```python
import os as _os
_os.environ.setdefault("JAX_PLATFORMS", "cpu")
import jax
import jax.numpy as jnp

def _softmax(x, axis=-1):
    return jax.nn.softmax(x, axis=axis)
def _gelu(x):
    return jax.nn.gelu(x, approximate=True)
def _silu(x):
    return jax.nn.silu(x)
def _sigmoid(x):
    return jax.nn.sigmoid(x)
def _layernorm(x, axis=-1, eps=1e-5):
    m = jnp.mean(x, axis=axis, keepdims=True)
    v = jnp.var(x, axis=axis, keepdims=True)
    return (x - m) / jnp.sqrt(v + eps)
def _scatter_add(tgt, idx, src, axis=0):
    return tgt.at[idx].add(src)
def _segment_sum(src, seg, n):
    return jax.ops.segment_sum(src, seg, n)
class _Rng:
    def __init__(self, key):
        self._k = key
    def _next(self):
        self._k, sub = jax.random.split(self._k)
        return sub
    def normal(self, shape):
        return jax.random.normal(self._next(), shape, dtype=jnp.bfloat16)
    def randint(self, lo, hi, shape):
        return jax.random.randint(self._next(), shape, lo, hi, dtype=jnp.int32)
    def uniform(self, shape, lo=0.0, hi=1.0):
        return jax.random.uniform(self._next(), shape, jnp.bfloat16, lo, hi)
    def permutation(self, n):
        return jax.random.permutation(self._next(), n)


kernel_name = 'sequential_preLN__mha_block__dense_activation_squared_relu__prompt'

def setup_inputs():
    _rng = _Rng(jax.random.key(int.from_bytes(__import__("os").urandom(4), "little")))
    _w = (lambda a: (lambda t: t.astype(jnp.bfloat16) if jnp.issubdtype(t.dtype, jnp.floating) else t)(jnp.asarray(a)))
    def _A_setup():
        B, S, D, H = 1, 2048, 448, 16
        return {
            "x": _w((lambda *s: _rng.normal(s) * 0.05)(B, S, D)),
            "wqkv": _w((lambda *s: _rng.normal(s) * 0.05)(D, 3 * D)),
            "wo": _w((lambda *s: _rng.normal(s) * 0.05)(D, D)),
        }
    _A_in = _A_setup()

    def _B_setup():
        B, S, D, F = 1, 2048, 448, 1792
        return {
            "x": _w((lambda *s: _rng.normal(s) * 0.05)(B, S, D)),
            "w1": _w((lambda *s: _rng.normal(s) * 0.05)(D, F)),
            "b1": _w((lambda *s: _rng.normal(s) * 0.05)(F)),
            "w2": _w((lambda *s: _rng.normal(s) * 0.05)(F, D)),
            "b2": _w((lambda *s: _rng.normal(s) * 0.05)(D)),
        }
    _B_in = _B_setup()

    return {
        "A_x": _A_in["x"],
        "A_wqkv": _A_in["wqkv"],
        "A_wo": _A_in["wo"],
        "B_x": _B_in["x"],
        "B_w1": _B_in["w1"],
        "B_b1": _B_in["b1"],
        "B_w2": _B_in["w2"],
        "B_b2": _B_in["b2"],
    }

def reference(A_x, A_wqkv, A_wo, B_x, B_w1, B_b1, B_w2, B_b2):
    def _A_ref(x, wqkv, wo):
        B, S, D = x.shape
        H = 16
        Dh = D // H
        qkv = (lambda x, *d: x.transpose(*d))((x @ wqkv).reshape(B, S, 3, H, Dh), 2, 0, 3, 1, 4)
        q, k, v = qkv[0], qkv[1], qkv[2]
        scores = jnp.einsum("bhqd,bhkd->bhqk", q, k) * (Dh ** -0.5)
        p = _softmax(scores, axis=-1)
        o = jnp.einsum("bhqk,bhkd->bhqd", p, v)
        return (lambda x, *d: x.transpose(*d))(o, 0, 2, 1, 3).reshape(B, S, D) @ wo

    def _B_ref(x, w1, b1, w2, b2):
        h = jnp.einsum("bsd,df->bsf", x, w1) + b1
        zero = jnp.zeros_like(h)
        r = jnp.where(h > zero, h, zero)
        h = r * r
        out = jnp.einsum("bsf,fd->bsd", h, w2) + b2
        return out

    x = A_x
    h = x + _A_ref(_layernorm(x, axis=-1), A_wqkv, A_wo)
    h2 = h + _B_ref(_layernorm(h, axis=-1), B_w1, B_b1, B_w2, B_b2)
    return h2
```

```python
import functools
import jax
import jax.numpy as jnp
from jax import lax
import jax.experimental.pallas as pl
import jax.experimental.pallas.tpu as pltpu

S, D, H, DH, F = 2048, 448, 16, 28, 1792
HP = 32
GW = 4 * DH
DA = 464
TQ = 512
NT = S // TQ
CK = 128
NC = S // CK
FC = 256
U = 4
EPS = 1e-5
QSCALE = (DH ** -0.5) * 1.4426950408889634
NEG = -1e30
F32 = jnp.float32
BF16 = jnp.bfloat16


def _pad_heads_rows(m, filler):
    parts = []
    for h in range(H):
        parts.append(m[DH * h:DH * (h + 1), :])
        parts.append(filler)
    return jnp.concatenate(parts, axis=0)


def _ln_cols(v):
    mu = jnp.mean(v, axis=0, keepdims=True)
    vc = v - mu
    var = jnp.mean(vc * vc, axis=0, keepdims=True)
    return vc * lax.rsqrt(var + EPS)


def _kernel(xT_hbm, wqkv_hbm, wo_hbm, w1_hbm, b1_hbm, w2T_hbm, b2_hbm, out_hbm,
            xT_s, wqkv_s, wo_s, w1_s, b1_s, w2T_s, b2_s,
            wT_s, woT_s, w1T_s, b2c_s, xn_s,
            k_s, qT_s, vT_s, s0, s1, oT_s, out_s, zero_s, sems):
    cp_wqkv = pltpu.make_async_copy(wqkv_hbm, wqkv_s, sems.at[0])
    cp_x0 = pltpu.make_async_copy(xT_hbm.at[0, :, pl.ds(0, TQ)], xT_s.at[:, pl.ds(0, TQ)], sems.at[1])
    cp_x1 = pltpu.make_async_copy(xT_hbm.at[0, :, pl.ds(TQ, S - TQ)], xT_s.at[:, pl.ds(TQ, S - TQ)], sems.at[2])
    cp_wo = pltpu.make_async_copy(wo_hbm, wo_s, sems.at[3])
    cp_w1 = pltpu.make_async_copy(w1_hbm, w1_s.at[pl.ds(0, D), :], sems.at[4])
    cp_b1 = pltpu.make_async_copy(b1_hbm, b1_s, sems.at[5])
    cp_w2 = pltpu.make_async_copy(w2T_hbm, w2T_s, sems.at[6])
    cp_b2 = pltpu.make_async_copy(b2_hbm, b2_s, sems.at[7])
    cp_x0.start()
    cp_wqkv.start()
    zero_s[0] = 0
    qT_s[pl.ds(D, DA - D), :] = jnp.zeros((DA - D, S), BF16)

    def ln1(c):
        xn_s[:, pl.ds(c * TQ, TQ)] = _ln_cols(xT_s[:, pl.ds(c * TQ, TQ)].astype(F32)).astype(BF16)

    frow = lax.broadcasted_iota(jnp.int32, (HP - DH, TQ), 0)
    vfill = jnp.where(frow == 0, 1.0, 0.0)

    def proj_q(c):
        cols = pl.ds(c * TQ, TQ)
        qT = jnp.dot(wT_s[pl.ds(0, D), :], xn_s[:, cols], preferred_element_type=F32)
        qT_s[pl.ds(0, D), cols] = (qT * QSCALE).astype(BF16)

    def proj_kv(c):
        cols = pl.ds(c * TQ, TQ)
        kv = jnp.dot(wT_s[pl.ds(D, 2 * D), :], xn_s[:, cols], preferred_element_type=F32)
        for g in range(4):
            k_s[g, cols, :] = kv[GW * g:GW * g + 128, :].astype(BF16).T
        vT_s[:, cols] = _pad_heads_rows(kv[D:, :], vfill).astype(BF16)

    cp_x0.wait()
    cp_x1.start()
    ln1(0)
    cp_wqkv.wait()
    cp_wo.start(); cp_w1.start(); cp_b1.start(); cp_b2.start()
    wT_s[...] = wqkv_s[...].T
    proj_kv(0)
    cp_x1.wait()
    cp_w2.start()
    ln1(1)
    proj_q(0)
    ln1(2)
    proj_kv(1)
    proj_q(1)
    ln1(3)
    proj_kv(2)
    proj_q(2)
    cp_wo.wait(); cp_w1.wait(); cp_b1.wait(); cp_b2.wait(); cp_w2.wait()
    proj_kv(3)
    proj_q(3)
    woT_s[...] = _pad_heads_rows(wo_s[...].astype(F32), jnp.zeros((HP - DH, D), F32)).astype(BF16).T
    brow = lax.broadcasted_iota(jnp.int32, (DA - D, F), 0)
    b1r = b1_s[...].astype(F32).reshape(1, F)
    w1_s[pl.ds(D, DA - D), :] = jnp.where(brow == 0, b1r, 0.0).astype(BF16)
    w1T_s[...] = w1_s[...].T
    b2c_s[...] = jnp.broadcast_to(b2_s[...].astype(F32).reshape(1, D), (128, D)).T

    zero = pl.multiple_of(zero_s[0], 8)
    qrow = lax.broadcasted_iota(jnp.int32, (128, TQ), 0)

    def q_weights(n, j):
        t = n // H
        g = (n % H) // 4
        q = qT_s[pl.ds(pl.multiple_of(g * GW, 16), 128), pl.ds(pl.multiple_of(t * TQ, TQ), TQ)].astype(F32)
        return jnp.where((qrow >= DH * j) & (qrow < DH * (j + 1)), q, 0.0).astype(BF16), g

    def a_chunk(g, qm, c, s_dst, m8):
        s = jnp.dot(k_s[g, pl.ds(c * CK, CK), :], qm, preferred_element_type=F32)
        s_dst[pl.ds(c * CK, CK), :] = s
        return jnp.maximum(m8, jnp.max(s.reshape(CK // 8, 8, TQ), axis=0))

    def bc_chunk(h, c, s_src, m, acc):
        p = jnp.exp2(s_src[pl.ds(zero + c * CK, CK), :] - m).astype(BF16)
        v = vT_s[pl.ds(pl.multiple_of(h * HP, HP), HP), pl.ds(c * CK, CK)]
        return acc + jnp.dot(v, p, preferred_element_type=F32)

    def fused(nA, jA, s_dst, hB, s_src, mB):
        qm, g = q_weights(nA, jA)
        m8 = jnp.full((8, TQ), NEG, F32)
        acc = jnp.zeros((HP, TQ), F32)
        for c in range(NC):
            m8 = a_chunk(g, qm, c, s_dst, m8)
            acc = bc_chunk(hB, c, s_src, mB, acc)
        o = acc * (1.0 / acc[DH:DH + 1, :])
        oT_s[pl.ds(pl.multiple_of(hB * HP, HP), HP), :] = o.astype(BF16)
        return jnp.max(m8, axis=0, keepdims=True)

    def out_copy(t):
        return pltpu.make_async_copy(out_s.at[t], out_hbm.at[0, :, pl.ds(pl.multiple_of(t * TQ, TQ), TQ)], sems.at[8 + t])

    def dense(t):
        cols = pl.ds(pl.multiple_of(t * TQ, TQ), TQ)
        hT = xT_s[:, cols].astype(F32) + jnp.dot(woT_s[...], oT_s[...], preferred_element_type=F32)
        hn = _ln_cols(hT).astype(BF16)
        arow = lax.broadcasted_iota(jnp.int32, (DA - D, TQ), 0)
        hn = jnp.concatenate([hn, jnp.where(arow == 0, 1.0, 0.0).astype(BF16)], axis=0)
        b2c = b2c_s[...]
        acc = hT + jnp.concatenate([b2c] * (TQ // 128), axis=1)
        for fc in range(F // FC):
            a = jnp.dot(w1T_s[pl.ds(fc * FC, FC), :], hn, preferred_element_type=F32)
            a = jnp.maximum(a, 0.0)
            a = (a * a).astype(BF16)
            acc = acc + jnp.dot(w2T_s[:, pl.ds(fc * FC, FC)], a, preferred_element_type=F32)
        out_s[t] = acc.astype(BF16)
        out_copy(t).start()

    qm, g = q_weights(0, 0)
    m8 = jnp.full((8, TQ), NEG, F32)
    for c in range(NC):
        m8 = a_chunk(g, qm, c, s0, m8)
    m0 = jnp.max(m8, axis=0, keepdims=True)

    def body(nb, m):
        for u in range(U):
            n = U * nb + u
            bufs = (s0, s1) if u % 2 == 0 else (s1, s0)
            nA = n + 1 if u < U - 1 else jnp.minimum(n + 1, NT * H - 4)
            m = fused(nA, (u + 1) % 4, bufs[1], n % H, bufs[0], m)

        @pl.when(nb % (H // U) == H // U - 1)
        def _():
            dense(nb // (H // U))
        return m

    lax.fori_loop(0, NT * H // U, body, m0)
    for t in range(NT):
        out_copy(t).wait()


@jax.jit
def pallas_sequential_preLN__mha_block__dense_activation_squared_relu__prompt_kernel(A_x, A_wqkv, A_wo, B_x, B_w1, B_b1, B_w2, B_b2):
    del B_x
    hbm = pl.BlockSpec(memory_space=pltpu.HBM)
    outT = pl.pallas_call(
        _kernel,
        out_shape=jax.ShapeDtypeStruct((1, D, S), BF16),
        in_specs=[hbm] * 7,
        out_specs=hbm,
        scratch_shapes=[
            pltpu.VMEM((D, S), BF16),
            pltpu.VMEM((D, 3 * D), BF16),
            pltpu.VMEM((D, D), BF16),
            pltpu.VMEM((DA, F), BF16),
            pltpu.VMEM((F,), BF16),
            pltpu.VMEM((D, F), BF16),
            pltpu.VMEM((D,), BF16),
            pltpu.VMEM((3 * D, D), BF16),
            pltpu.VMEM((D, H * HP), BF16),
            pltpu.VMEM((F, DA), BF16),
            pltpu.VMEM((D, 128), F32),
            pltpu.VMEM((D, S), BF16),
            pltpu.VMEM((4, S, 128), BF16),
            pltpu.VMEM((DA, S), BF16),
            pltpu.VMEM((H * HP, S), BF16),
            pltpu.VMEM((S, TQ), F32),
            pltpu.VMEM((S, TQ), F32),
            pltpu.VMEM((H * HP, TQ), BF16),
            pltpu.VMEM((NT, D, TQ), BF16),
            pltpu.SMEM((1,), jnp.int32),
            pltpu.SemaphoreType.DMA((12,)),
        ],
        compiler_params=pltpu.CompilerParams(vmem_limit_bytes=100 * 1024 * 1024),
        name="fused_block",
    )(jnp.transpose(A_x, (0, 2, 1)), A_wqkv, A_wo, B_w1, B_b1, B_w2.T, B_b2)
    return jnp.transpose(outT, (0, 2, 1))
```

```python
import jax
import jax.numpy as jnp
from jax import lax
import jax.experimental.pallas as pl
import jax.experimental.pallas.tpu as pltpu

S, D, H, DH, F = 2048, 448, 16, 28, 1792
HP = 32
GW = 4 * DH
DA = 464
PC = 512
TQ = 256
NT = S // TQ
HPI = 2
NI = H // HPI
SW = HPI * TQ
CK = 128
NC = S // CK
LAG = 4
LW = 128
NG = TQ // LW
KP = 3 * 128
UR = 64
FILL = (0, 1, 0, 1, 1, 1, 0, 0, 1, 1, 1, 0, 0, 1, 0, 1)
T1, T2 = 4, 192
FCH = ((0, 512), (512, 512), (1024, 512), (1536, 256))
OR = 224
WA1, WA, XA = 256, 512, 256
QA, QS, VS = 224, 368, 384
EPS = 1e-5
QSCALE = (DH ** -0.5) * 1.4426950408889634
F32 = jnp.float32
BF16 = jnp.bfloat16
U32 = jnp.uint32


def _pad_heads_rows(m, filler):
    parts = []
    for h in range(H):
        parts.append(m[DH * h:DH * (h + 1), :])
        parts.append(filler)
    return jnp.concatenate(parts, axis=0)


def _fold(v):
    v = jnp.sum(v.reshape(v.shape[0] // 16, 16, v.shape[1]), axis=0)
    return v[:8] + v[8:]


def _colmean(parts):
    return jnp.sum((parts[0] + parts[1]) + (parts[2] + parts[3]), axis=0, keepdims=True) * (1.0 / D)


def _pk(x):
    return pltpu.bitcast(x, U32)


def _up(x):
    return pltpu.bitcast(x, BF16)


def _h(start, size):
    return pl.ds(start // 2, size // 2)


def _dot(a, b):
    return jnp.dot(a, b, preferred_element_type=F32)


def _kernel(xT_hbm, wqkv_hbm, wo_hbm, w1_hbm, b1_hbm, w2T_hbm, b2_hbm, out_hbm,
            xT_s, wqkv_s, wo_s, w1_s, b1_s, w2T_s, b2_s,
            wT_s, woT_s, w1T_s, b2c_s, xn_s,
            k_s, qT_s, qc_s, vT_s, s0, s1, s2, oT_s, hn_s, out_s, zero_s, dz_s, sems, *hbufs):
    def w_copy(c0, n, sem):
        return pltpu.make_async_copy(wqkv_hbm.at[:, pl.ds(c0, n)], wqkv_s.at[:, pl.ds(c0, n)], sems.at[sem])

    def x_copy(c0, n, sem):
        return pltpu.make_async_copy(xT_hbm.at[0, :, pl.ds(c0, n)], xT_s.at[:, pl.ds(c0, n)], sems.at[sem])

    grp_a = [w_copy(0, WA1, 0), x_copy(0, XA, 0)]
    grp_b = [x_copy(XA, PC - XA, 1), w_copy(WA1, WA - WA1, 1)]
    grp_c = [w_copy(2 * D, D, 3)]
    grp_d = [w_copy(WA, 2 * D - WA, 2), x_copy(PC, PC, 2)]
    grp_e = [x_copy(2 * PC, 2 * PC, 4),
             pltpu.make_async_copy(wo_hbm, wo_s, sems.at[4]),
             pltpu.make_async_copy(w1_hbm, w1_s.at[pl.ds(0, D), :], sems.at[4]),
             pltpu.make_async_copy(b1_hbm, b1_s, sems.at[4]),
             pltpu.make_async_copy(b2_hbm, b2_s, sems.at[4])]
    grp_f = [pltpu.make_async_copy(w2T_hbm, w2T_s, sems.at[0])]

    def start(grp):
        for cp in grp:
            cp.start()

    def wait(grp):
        for cp in grp:
            cp.wait()

    start(grp_a)
    start(grp_b)
    for k in range(3):
        zero_s[k] = 0
        dz_s[k] = 0
    zeros = [pl.multiple_of(zero_s[k], 16) for k in range(3)]
    qT_s[_h(D, DA - D), :] = jnp.zeros(((DA - D) // 2, S), U32)
    arow = lax.broadcasted_iota(jnp.int32, (DA - D, TQ), 0)
    hn_s[_h(D, DA - D), :] = _pk(jnp.where(arow == 0, 1.0, 0.0).astype(BF16))

    def ln1(c0, c1, split=False):
        for cg in range(c0 // LW, c1 // LW):
            cols = pl.ds(cg * LW, LW)
            if split:
                ld = lambda k, r: xT_s[pl.ds(zeros[k] + r * GW, GW), cols].astype(F32)
                mu = _colmean([_fold(ld(0, r)) for r in range(4)])
                var = _colmean([_fold(jnp.square(ld(1, r) - mu)) for r in range(4)])
                rs = lax.rsqrt(var + EPS)
                for r in range(4):
                    xn_s[_h(r * GW, GW), cols] = _pk(((ld(2, r) - mu) * rs).astype(BF16))
            else:
                ld = lambda k: xT_s[pl.ds(zeros[k], D), cols].astype(F32)
                mu = jnp.sum(ld(0), axis=0, keepdims=True) * (1.0 / D)
                var = jnp.sum(jnp.square(ld(1) - mu), axis=0, keepdims=True) * (1.0 / D)
                xn_s[:, cols] = _pk(((ld(2) - mu) * lax.rsqrt(var + EPS)).astype(BF16))

    def w_transpose(c0, n):
        wT_s[_h(c0, n), :] = _pk(wqkv_s[:, pl.ds(c0, n)].T)

    def proj(r0, nr, c0, c1):
        return _dot(_up(wT_s[_h(r0, nr), :]), _up(xn_s[:, pl.ds(c0, c1 - c0)]))

    def put_k(kT, c0):
        for g in range(4):
            k_s[g, _h(c0, PC), :] = _pk(kT[GW * g:GW * g + 128, :].astype(BF16).T)

    def put_v(vT, c0, c1):
        ones_row = jnp.where(lax.broadcasted_iota(jnp.int32, (HP - DH, c1 - c0), 0) == 0, 1.0, 0.0)
        vT_s[:, pl.ds(c0, c1 - c0)] = _pk(_pad_heads_rows(vT, ones_row).astype(BF16))

    def proj_q(c0, c1, r0=0, r1=D):
        qT_s[_h(r0, r1 - r0), pl.ds(c0, c1 - c0)] = _pk((proj(r0, r1 - r0, c0, c1) * QSCALE).astype(BF16))

    def proj_kv(c0):
        kv = proj(D, 2 * D, c0, c0 + PC)
        put_k(kv, c0)
        put_v(kv[D:, :], c0, c0 + PC)

    def prologue():
        wait(grp_a)
        start(grp_c)
        start(grp_d)
        for c0 in range(0, WA1, 128):
            w_transpose(c0, 128)
        ln1(0, XA, True)
        proj_q(0, XA, 0, QA)
        wait(grp_b)
        for c0 in range(WA1, WA, 128):
            w_transpose(c0, 128)
        ln1(XA, XA + LW, True)
        proj_q(0, XA, QA, WA1)
        ln1(XA + LW, PC)
        proj_q(0, XA, WA1, QS)
        proj_q(XA, PC, 0, QS)
        wait(grp_c)
        start(grp_e)
        w_transpose(2 * D, D)
        proj_q(0, PC, QS, D)
        put_v(proj(2 * D, D, 0, VS), 0, VS)
        wait(grp_d)
        start(grp_f)
        w_transpose(WA, 2 * D - WA)
        put_v(proj(2 * D, D, VS, PC), VS, PC)
        ln1(PC, 2 * PC)
        put_k(jnp.concatenate([proj(D, D, 0, PC), jnp.zeros((DA - D, PC), F32)], axis=0), 0)
        proj_kv(PC)
        wait(grp_e)
        ln1(2 * PC, 3 * PC)
        proj_q(PC, 2 * PC)
        ln1(3 * PC, 4 * PC)
        proj_kv(2 * PC)
        proj_q(2 * PC, 3 * PC)
        proj_kv(3 * PC)
        proj_q(3 * PC, 4 * PC)
        woT_s[...] = _pk(_pad_heads_rows(wo_s[...].astype(F32), jnp.zeros((HP - DH, D), F32)).astype(BF16).T)
        brow = lax.broadcasted_iota(jnp.int32, (DA - D, F), 0)
        w1_s[pl.ds(D, DA - D), :] = jnp.where(brow == 0, b1_s[...].astype(F32).reshape(1, F), 0.0).astype(BF16)
        w1T_s[...] = _pk(w1_s[...].T)
        b2c_s[...] = jnp.broadcast_to(b2_s[...].astype(F32).reshape(1, D), (LW, D)).T
        qc_s[...] = qT_s[:, pl.ds(0, TQ)]
        wait(grp_f)

    zero = zeros[0]
    qrow = lax.broadcasted_iota(jnp.int32, (128, TQ), 0)
    bufs = (s0, s1, s2)
    h_s, hp_s = hbufs[:NG], hbufs[NG:]

    def out_copy(t, og):
        return pltpu.make_async_copy(out_s.at[t, pl.ds(og * OR, OR), :],
                                     out_hbm.at[0, pl.ds(og * OR, OR), pl.ds(pl.multiple_of(t * TQ, TQ), TQ)],
                                     sems.at[5])

    def tile(t):
        col0 = pl.multiple_of(t * TQ, TQ)
        dz = [pl.multiple_of(dz_s[k], 16) for k in range(3)]
        st = {"m": {}}

        def scores(a):
            i, c = a // NC, a % NC
            g = (i * HPI) // 4
            if c == 0:
                q = _up(qc_s[_h(g * GW, 128), :]).astype(F32)
                js = [(i * HPI + k) % 4 for k in range(HPI)]
                st["qm"] = jnp.concatenate(
                    [jnp.where((qrow >= DH * j) & (qrow < DH * (j + 1)), q, 0.0) for j in js], axis=1).astype(BF16)
            s = _dot(_up(k_s[g, _h(c * CK, CK), :]), st["qm"])
            bufs[i % 3][pl.ds(c * CK, CK), :] = s
            m8 = jnp.max(s.reshape(CK // 8, 8, SW), axis=0)
            st["m8"] = m8 if c == 0 else jnp.maximum(st["m8"], m8)
            if c == NC - 1:
                st["m"][i] = jnp.max(st["m8"], axis=0, keepdims=True)

        def probs_pv(i, k0, nk, q0, nq):
            accs = []
            for k in range(HPI):
                h = i * HPI + k
                lo = k * TQ + q0
                p = jnp.exp2(bufs[i % 3][pl.ds(zero + k0, nk), pl.ds(lo, nq)] - st["m"][i][:, lo:lo + nq])
                pv = _dot(_up(vT_s[_h(h * HP, HP), pl.ds(k0, nk)]), p.astype(BF16))
                acc = pv if k0 == 0 else st["acc"][k] + pv
                accs.append(acc)
                if k0 + nk == S:
                    l = acc[DH:DH + 1, :]
                    r = pl.reciprocal(l, approx=True)
                    r = r * (2.0 - l * r)
                    oT_s[_h(h * HP, HP), pl.ds(q0, nq)] = _pk((acc * r).astype(BF16))
            st["acc"] = accs

        def wo_part(cg, r):
            rows = pl.ds(r * UR, UR)
            hp = (xT_s[rows, pl.ds(pl.multiple_of(col0 + cg * LW, LW), LW)].astype(F32)
                  + _dot(_up(woT_s[_h(r * UR, UR), pl.ds(0, KP)]), _up(oT_s[_h(0, KP), pl.ds(cg * LW, LW)])))
            hp_s[cg][rows, :] = hp
            st["c", cg] = _fold(hp) if r == 0 else st["c", cg] + _fold(hp)

        def wo_last_ln2(cg):
            lc = pl.ds(cg * LW, LW)
            ol = _up(oT_s[_h(KP, H * HP - KP), lc])
            shift = jnp.sum(st["c", cg], axis=0, keepdims=True) * (1.0 / D)
            p1, p2 = [], []
            for r in range(4):
                hr = (hp_s[cg][pl.ds(dz[0] + r * GW, GW), :]
                      + _dot(_up(woT_s[_h(r * GW, GW), pl.ds(KP, H * HP - KP)]), ol))
                h_s[cg][pl.ds(r * GW, GW), :] = hr
                d = hr - shift
                p1.append(_fold(d))
                p2.append(_fold(d * d))
            dm = _colmean(p1)
            rs = lax.rsqrt(jnp.maximum(_colmean(p2) - dm * dm, 0.0) + EPS)
            mu = shift + dm
            for r in range(4):
                hn_s[_h(r * GW, GW), lc] = _pk(((h_s[cg][pl.ds(dz[2] + r * GW, GW), :] - mu) * rs).astype(BF16))

        def ffn1(f0, fn, cg=None):
            hn = hn_s[...] if cg is None else hn_s[:, pl.ds(cg * LW, LW)]
            a = jnp.maximum(_dot(_up(w1T_s[_h(f0, fn), :]), _up(hn)), 0.0)
            return a * a

        queue = [(cg, r) for cg in range(NG) for r in range(D // UR)]

        def fill(n):
            for _ in range(min(n, len(queue))):
                wo_part(*queue.pop(0))

        for a in range(NI * NC + LAG):
            b = a - NC - LAG
            if b >= 0:
                probs_pv(b // NC, (b % NC) * CK, CK, 0, TQ)
            if a < NI * NC:
                scores(a)
            else:
                fill(1)
        nch = NC // NG
        for cg in range(NG):
            for c in range(nch):
                if cg > 0 and c == T1:
                    wo_last_ln2(cg - 1)
                probs_pv(NI - 1, c * CK * NG, CK * NG, cg * LW, LW)
                fill(FILL[cg * nch + c])
        fill(len(queue))
        f0, fn = FCH[0]
        a00 = ffn1(f0, T2, 0)
        wo_last_ln2(NG - 1)
        a01 = ffn1(f0 + T2, fn - T2, 0)
        a_next = jnp.concatenate([jnp.concatenate([a00, a01], axis=0), ffn1(f0, fn, 1)], axis=1)

        qc_s[...] = qT_s[:, pl.ds(pl.multiple_of(jnp.minimum(t + 1, NT - 1) * TQ, TQ), TQ)]
        b2c = b2c_s[...]
        acc = jnp.concatenate([h_s[cg][pl.ds(dz[0], D), :] + b2c for cg in range(NG)], axis=1)
        for i, (f0, fn) in enumerate(FCH):
            a = a_next.astype(BF16)
            if i < len(FCH) - 1:
                a_next = ffn1(*FCH[i + 1])
                acc = acc + _dot(w2T_s[:, pl.ds(f0, fn)], a)
            else:
                for og in range(D // OR):
                    res = acc[og * OR:(og + 1) * OR, :] + _dot(w2T_s[pl.ds(og * OR, OR), pl.ds(f0, fn)], a)
                    out_s[t, pl.ds(og * OR, OR), :] = res.astype(BF16)
                    out_copy(t, og).start()

    def step(i, carry):
        pl.when(i == 0)(prologue)
        pl.when(i > 0)(lambda: tile(i - 1))
        return carry

    lax.fori_loop(0, NT + 1, step, 0)
    for t in range(NT):
        for og in range(D // OR):
            out_copy(t, og).wait()


@jax.jit
def pallas_sequential_preLN__mha_block__dense_activation_squared_relu__prompt_kernel(
    A_x: jax.Array,
    A_wqkv: jax.Array,
    A_wo: jax.Array,
    B_x: jax.Array,
    B_w1: jax.Array,
    B_b1: jax.Array,
    B_w2: jax.Array,
    B_b2: jax.Array,
):
    del B_x
    hbm = pl.BlockSpec(memory_space=pltpu.HBM)
    outT = pl.pallas_call(
        _kernel,
        out_shape=jax.ShapeDtypeStruct((1, D, S), BF16),
        in_specs=[hbm] * 7,
        out_specs=hbm,
        scratch_shapes=[
            pltpu.VMEM((D, S), BF16),
            pltpu.VMEM((D, 3 * D), BF16),
            pltpu.VMEM((D, D), BF16),
            pltpu.VMEM((DA, F), BF16),
            pltpu.VMEM((F,), BF16),
            pltpu.VMEM((D, F), BF16),
            pltpu.VMEM((D,), BF16),
            pltpu.VMEM((3 * D // 2, D), U32),
            pltpu.VMEM((D // 2, H * HP), U32),
            pltpu.VMEM((F // 2, DA), U32),
            pltpu.VMEM((D, LW), F32),
            pltpu.VMEM((D // 2, S), U32),
            pltpu.VMEM((4, S // 2, 128), U32),
            pltpu.VMEM((DA // 2, S), U32),
            pltpu.VMEM((DA // 2, TQ), U32),
            pltpu.VMEM((H * HP // 2, S), U32),
            pltpu.VMEM((S, SW), F32),
            pltpu.VMEM((S, SW), F32),
            pltpu.VMEM((S, SW), F32),
            pltpu.VMEM((H * HP // 2, TQ), U32),
            pltpu.VMEM((DA // 2, TQ), U32),
            pltpu.VMEM((NT, D, TQ), BF16),
            pltpu.SMEM((3,), jnp.int32),
            pltpu.SMEM((3,), jnp.int32),
            pltpu.SemaphoreType.DMA((6,)),
        ] + [pltpu.VMEM((D, LW), F32)] * (2 * NG),
        compiler_params=pltpu.CompilerParams(vmem_limit_bytes=100 * 1024 * 1024,
                                             disable_bounds_checks=True,
                                             disable_semaphore_checks=True),
        name="fused_block",
    )(jnp.transpose(A_x, (0, 2, 1)), A_wqkv, A_wo, B_w1, B_b1, B_w2.T, B_b2)
    return jnp.transpose(outT, (0, 2, 1))
```

```python
import jax
import jax.numpy as jnp
from jax import lax
import jax.experimental.pallas as pl
import jax.experimental.pallas.tpu as pltpu

S, D, H, DH, F = 2048, 448, 16, 28, 1792
HP = 32
GW = 4 * DH
DA = 464
PC = 512
TQ = 256
NT = S // TQ
HPI = 2
NI = H // HPI
SW = HPI * TQ
CK = 128
NC = S // CK
LAG = 3
LW = 128
NG = TQ // LW
NLT = SW // LW
KP = 3 * 128
UR = 64
FCH = ((0, 512), (512, 512), (1024, 512), (1536, 256))
OR = 224
FILL = (0, 1, 0, 1, 1, 1, 0, 0, 1, 1, 1, 0, 0, 1, 0, 1)
T1, T2, ROT = 5, 160, 2
W0, W1, XA = 384, 640, 256
KA, KS, VS = 576, 720, 384
TB1, TB2 = 23, 160
NV, UK = 192, 16
NKG = NV // UK
NCH = NLT * NKG
RP = (2, 1, 2, 2, 3, 1, 2, 2, 3, 2, 2, 2, 2, 2, 2, 2)
RATE = [2 if a < NC + LAG else (RP[a % NC] if a < NI * NC - 4 else 0) for a in range(NI * NC)]
NA = NI * NCH - sum(RATE)
PA, PL = -(-NA // NCH), NA // NCH
QLO, QHI = -(-PA * HPI * DH // 16) * 16, PL * HPI * DH // 16 * 16
FW = (0, 0.7, 1, 1, 1.15, 1, 1, 1, 1, 0.5, 0)
TD, FD = 2, 32
MCH = [NV + 16 * (c * ((S - NV) // 16) // NC) for c in range(NC + 1)]
EPS = 1e-5
QSCALE = (DH ** -0.5) * 1.4426950408889634
LOWEST = -3.0e38
F32 = jnp.float32
BF16 = jnp.bfloat16
U32 = jnp.uint32


def _pad_heads_rows(m, filler):
    parts = []
    for h in range(H):
        parts.append(m[DH * h:DH * (h + 1), :])
        parts.append(filler)
    return jnp.concatenate(parts, axis=0)


def _fold(v):
    v = jnp.sum(v.reshape(v.shape[0] // 16, 16, v.shape[1]), axis=0)
    return v[:8] + v[8:]


def _colmean(parts):
    return jnp.sum((parts[0] + parts[1]) + (parts[2] + parts[3]), axis=0, keepdims=True) * (1.0 / D)


def _pk(x):
    return pltpu.bitcast(x, U32)


def _up(x):
    return pltpu.bitcast(x, BF16)


def _h(start, size):
    return pl.ds(start // 2, size // 2)


def _dot(a, b):
    return jnp.dot(a, b, preferred_element_type=F32)


def _unit(u):
    return u % NLT, (u // NLT + 4 * (u % NLT)) % NKG


def _kernel(xT_hbm, wqkv_hbm, wo_hbm, w1_hbm, b1_hbm, w2T_hbm, b2_hbm, out_hbm,
            xT_s, wqkv_s, wo_s, w1_s, b1_s, w2T_s, b2_s,
            wT_s, woT_s, w1T_s, b2c_s, xn_s,
            k_s, kb_s, qT_s, qc_s, qf_s, qn_s, vT_s, s0, s1, s2, sv_s, oT_s, hn_s, out_s,
            zero_s, dz_s, sems, *hbufs):
    def w_copy(c0, n, sem):
        return pltpu.make_async_copy(wqkv_hbm.at[:, pl.ds(c0, n)], wqkv_s.at[:, pl.ds(c0, n)], sems.at[sem])

    def x_copy(c0, n, sem):
        return pltpu.make_async_copy(xT_hbm.at[0, :, pl.ds(c0, n)], xT_s.at[:, pl.ds(c0, n)], sems.at[sem])

    grp_a = [w_copy(W0, W1 - W0, 0), x_copy(0, XA, 0)]
    grp_b = [x_copy(XA, PC - XA, 1), w_copy(W1, 2 * D - W1, 1)]
    grp_c = [w_copy(0, W0, 3)]
    grp_d = [w_copy(2 * D, D, 2), x_copy(PC, PC, 2)]
    grp_e = [x_copy(2 * PC, 2 * PC, 4),
             pltpu.make_async_copy(wo_hbm, wo_s, sems.at[4]),
             pltpu.make_async_copy(w1_hbm, w1_s.at[pl.ds(0, D), :], sems.at[4]),
             pltpu.make_async_copy(b1_hbm, b1_s, sems.at[4]),
             pltpu.make_async_copy(b2_hbm, b2_s, sems.at[4])]
    grp_f = [pltpu.make_async_copy(w2T_hbm, w2T_s, sems.at[0])]

    def start(grp):
        for cp in grp:
            cp.start()

    def wait(grp):
        for cp in grp:
            cp.wait()

    start(grp_a)
    start(grp_b)
    for k in range(3):
        zero_s[k] = 0
        dz_s[k] = 0
    zeros0 = [pl.multiple_of(zero_s[k], 16) for k in range(3)]
    zero = zeros0[0]
    qT_s[_h(D, DA - D), :] = jnp.zeros(((DA - D) // 2, S), U32)
    arow = lax.broadcasted_iota(jnp.int32, (DA - D, TQ), 0)
    hn_s[_h(D, DA - D), :] = _pk(jnp.where(arow == 0, 1.0, 0.0).astype(BF16))

    def ln1(c0, c1, split=False):
        zeros = zeros0 if split else [pl.multiple_of(dz_s[k], 16) for k in range(3)]
        for cg in range(c0 // LW, c1 // LW):
            cols = pl.ds(cg * LW, LW)
            if split:
                ld = lambda k, r: xT_s[pl.ds(zeros[k] + r * GW, GW), cols].astype(F32)
                mu = _colmean([_fold(ld(0, r)) for r in range(4)])
                var = _colmean([_fold(jnp.square(ld(1, r) - mu)) for r in range(4)])
                rs = lax.rsqrt(var + EPS)
                for r in range(4):
                    xn_s[_h(r * GW, GW), cols] = _pk(((ld(2, r) - mu) * rs).astype(BF16))
            else:
                ld = lambda k: xT_s[pl.ds(zeros[k], D), cols].astype(F32)
                mu = jnp.sum(ld(0), axis=0, keepdims=True) * (1.0 / D)
                var = jnp.sum(jnp.square(ld(1) - mu), axis=0, keepdims=True) * (1.0 / D)
                xn_s[:, cols] = _pk(((ld(2) - mu) * lax.rsqrt(var + EPS)).astype(BF16))

    def w_transpose(c0, n):
        wT_s[_h(c0, n), :] = _pk(wqkv_s[:, pl.ds(c0, n)].T)

    def k_table(d0, d1, gate=None):
        for g in range(4):
            lo, hi = max(d0, g * GW), min(d1, (g + 1) * GW)
            if lo >= hi:
                continue
            kp = k_s[g, pl.ds(zero, NV // 2), :]
            if gate is not None:
                kp = kp | pltpu.bitcast(gate - gate, U32)
            kb_s[pl.ds(lo, hi - lo)] = jnp.concatenate(
                [_up(jnp.broadcast_to(kp[:, d - g * GW:d - g * GW + 1], (NV // 2, 128))).astype(F32)[None]
                 for d in range(lo, hi)], axis=0)

    def proj(r0, r1, c0, c1):
        xr = pl.ds(zero if c0 >= PC else 0, D // 2)
        return _dot(_up(wT_s[_h(r0, r1 - r0), :]), _up(xn_s[xr, pl.ds(c0, c1 - c0)]))

    def put_q(z, r0, c0):
        qT_s[_h(r0, z.shape[0]), pl.ds(c0, z.shape[1])] = _pk((z * QSCALE).astype(BF16))

    def put_k(kT, c0):
        for g in range(4):
            k_s[g, _h(c0, kT.shape[1]), :] = _pk(kT[GW * g:GW * g + 128, :].astype(BF16).T)

    def put_v(vT, c0):
        ones_row = jnp.where(lax.broadcasted_iota(jnp.int32, (HP - DH, PC), 0) == 0, 1.0, 0.0)
        vT_s[:, pl.ds(c0, PC)] = _pk(_pad_heads_rows(vT, ones_row).astype(BF16))

    def proj_q(r0, r1, c0, c1):
        put_q(proj(r0, r1, c0, c1), r0, c0)

    def proj_kv(c0):
        kv = proj(D, 3 * D, c0, c0 + PC)
        put_k(kv, c0)
        put_v(kv[D:, :], c0)

    def load_q(cols, gate=None):
        q = qT_s[:, cols]
        qc_s[...] = q
        qf = _up(q[QHI // 2:D // 2]).astype(F32)
        if gate is not None:
            qf = qf + (gate - gate)
        qf_s[pl.ds(QHI, D - QHI), :] = qf

    qrow = lax.broadcasted_iota(jnp.int32, (128, TQ), 0)

    def qweights(i):
        q = _up(qc_s[_h((i * HPI) // 4 * GW, 128), :]).astype(F32)
        js = [(i * HPI + k) % 4 for k in range(HPI)]
        return jnp.concatenate(
            [jnp.where((qrow >= DH * j) & (qrow < DH * (j + 1)), q, 0.0) for j in js], axis=1).astype(BF16)

    def prologue():
        pk = lambda r0, r1, c0, c1: proj(r0, r1, c0, c1).astype(BF16)
        pad = lambda n: jnp.zeros((DA - D, n), BF16)
        wait(grp_a)
        start(grp_c)
        start(grp_d)
        for c0 in range(W0, W1, 128):
            w_transpose(c0, 128)
        ln1(0, XA, True)
        proj_q(W0, D, 0, XA)
        k1 = pk(D, KA, 0, XA)
        wait(grp_b)
        for c0 in range(W1, 2 * D, 128):
            w_transpose(c0, 128)
        ln1(XA, XA + LW, True)
        k2 = pk(KA, W1, 0, XA)
        ln1(XA + LW, PC)
        put_k(jnp.concatenate([k1, k2, pk(W1, 2 * D, 0, XA), pad(XA)], axis=0), 0)
        k3 = pk(D, KS, XA, PC)
        wait(grp_c)
        start(grp_e)
        w_transpose(0, W0)
        k_table(0, TB1)
        put_k(jnp.concatenate([k3, pk(KS, 2 * D, XA, PC), pad(PC - XA)], axis=0), XA)
        proj_q(W0, D, XA, PC)
        proj_q(0, W0, 0, VS)
        wait(grp_d)
        start(grp_f)
        w_transpose(2 * D, D)
        proj_q(0, W0, VS, PC)
        k_table(TB1, TB2)
        ln1(PC, 2 * PC)
        put_v(proj(2 * D, 3 * D, 0, PC), 0)
        proj_kv(PC)
        wait(grp_e)
        ln1(2 * PC, 3 * PC)
        z = proj(0, D, PC, 2 * PC)
        k_table(TB2, D, z[0:1, 0:LW])
        put_q(z, 0, PC)
        ln1(3 * PC, 4 * PC)
        proj_kv(2 * PC)
        proj_q(0, D, 2 * PC, 3 * PC)
        proj_kv(3 * PC)
        proj_q(0, D, 3 * PC, 4 * PC)
        woT_s[...] = _pk(_pad_heads_rows(wo_s[...].astype(F32), jnp.zeros((HP - DH, D), F32)).astype(BF16).T)
        brow = lax.broadcasted_iota(jnp.int32, (DA - D, F), 0)
        w1_s[pl.ds(D, DA - D), :] = jnp.where(brow == 0, b1_s[...].astype(F32).reshape(1, F), 0.0).astype(BF16)
        w1T_s[...] = _pk(w1_s[...].T)
        b2c_s[...] = jnp.broadcast_to(b2_s[...].astype(F32).reshape(1, D), (LW, D)).T
        load_q(pl.ds(0, TQ))
        for i in range(PA):
            sv_s[i] = _dot(_up(k_s[(i * HPI) // 4, _h(0, NV), :]), qweights(i))
        wait(grp_f)

    bufs = (s0, s1, s2)
    h_s, hp_s = hbufs[:NG], hbufs[NG:]

    def out_copy(t, og):
        return pltpu.make_async_copy(out_s.at[t, pl.ds(og * OR, OR), :],
                                     out_hbm.at[0, pl.ds(og * OR, OR), pl.ds(pl.multiple_of(t * TQ, TQ), TQ)],
                                     sems.at[5])

    def tile(t):
        col0 = pl.multiple_of(t * TQ, TQ)
        dz = [pl.multiple_of(dz_s[k], 16) for k in range(3)]
        st = {"m": {}, "pend": [], "ties": [], "fi": 0}

        nxt = pl.ds(pl.multiple_of(jnp.minimum(t + 1, NT - 1) * TQ, TQ), TQ)
        qn_s[pl.ds(zero, QLO), :] = _up(qT_s[_h(0, QLO), nxt]).astype(F32)
        units = [(i,) + _unit(u) + (i * NCH + u < NA,) for i in range(NI) for u in range(NCH)]
        units = units[NA:] + units[:NA]

        def vpu_unit(gate):
            i, lt, kg, ahead = units.pop(0)
            h = i * HPI + lt // NG
            if ("qv", i, lt, ahead) not in st:
                q_ref = qn_s if ahead else qf_s
                st["qv", i, lt, ahead] = jnp.concatenate(
                    [jnp.broadcast_to(q_ref[pl.ds(h * DH + d, 1), pl.ds(lt % NG * LW, LW)], (UK, LW))[None]
                     for d in range(DH)], axis=0)
            prod = kb_s[pl.ds(h * DH, DH), pl.ds(kg * UK, UK), :] * st["qv", i, lt, ahead]
            z0 = jnp.concatenate([gate - gate] * (UK // 8), axis=0)
            acc = jnp.sum(jnp.concatenate([z0[None], prod], axis=0), axis=0)
            sv_s[i, pl.ds(kg * UK, UK), pl.ds(lt * LW, LW)] = acc
            return jnp.minimum(jnp.min(acc.reshape(UK // 8, 8, LW), axis=0), LOWEST)

        def scores(a):
            i, c = a // NC, a % NC
            if c == 0:
                st["qm"] = qweights(i)
            k0, nk = MCH[c], MCH[c + 1] - MCH[c]
            s = _dot(_up(k_s[(i * HPI) // 4, _h(k0, nk), :]), st["qm"])
            bufs[i % 3][pl.ds(k0, nk), :] = s
            for lt in range(NLT):
                m = jnp.max(s[:, lt * LW:(lt + 1) * LW].reshape(nk // 8, 8, LW), axis=0)
                st["m8", lt] = m if c == 0 else jnp.maximum(m, st["m8", lt])
            pend = st["pend"]
            for j in range(RATE[a]):
                r, lt = j * (nk // 8) // RATE[a] + 1, 2 * j % NLT
                pend.append((a + TD, (lt + 2) % NLT, vpu_unit(s[8 * r:8 * r + 8, lt * LW:(lt + 1) * LW])))
            while pend and pend[0][0] <= a:
                _, lt, v = pend.pop(0)
                st["m8", lt] = jnp.maximum(st["m8", lt], v)
            for u in range(c * NCH // NC, (c + 1) * NCH // NC):
                lt, kg = _unit(u)
                assert (i, lt, kg, False) not in units
                sv = sv_s[i, pl.ds(zero + kg * UK, UK), pl.ds(lt * LW, LW)]
                st["m8", lt] = jnp.maximum(st["m8", lt], jnp.max(sv.reshape(UK // 8, 8, LW), axis=0))
            if c == NC - 1:
                m8 = jnp.concatenate([st["m8", lt] for lt in range(NLT)], axis=1)
                st["m"][i] = jnp.max(m8, axis=0, keepdims=True)

        def probs_pv(i, k0, nk, q0, nq, first, last):
            for k in range(HPI):
                h = i * HPI + k
                lo = k * TQ + q0
                parts = []
                if k0 < NV:
                    parts.append(sv_s[i, pl.ds(zero + k0, min(NV - k0, nk)), pl.ds(lo, nq)])
                if k0 + nk > NV:
                    parts.append(bufs[i % 3][pl.ds(zero + max(k0, NV), k0 + nk - max(k0, NV)), pl.ds(lo, nq)])
                p = jnp.exp2(jnp.concatenate(parts, axis=0) - st["m"][i][:, lo:lo + nq])
                pv = _dot(_up(vT_s[_h(h * HP, HP), pl.ds(k0, nk)]), p.astype(BF16))
                acc = pv if first else st["acc", k] + pv
                st["acc", k] = acc
                if last:
                    l = acc[DH:DH + 1, :]
                    r = pl.reciprocal(l, approx=True)
                    r = r * (2.0 - l * r)
                    oT_s[_h(h * HP, HP), pl.ds(q0, nq)] = _pk((acc * r).astype(BF16))

        fcost = [T2, FCH[0][1] - T2, FCH[0][1]]
        for idx, (f0, fn) in enumerate(FCH):
            if idx < len(FCH) - 1:
                fcost += [2 * FCH[idx + 1][1], D * fn // 256]
            else:
                fcost += [OR * fn // 256] * (D // OR)
        fcost = [c * w for c, w in zip(fcost, FW)]
        fcum = [int(sum(fcost[:j]) * NA / sum(fcost) + 1e-6) for j in range(len(fcost) + 1)]

        def fdot(a, b):
            if b.shape[0] > 256 and b.shape[1] > LW:
                z = jnp.concatenate([_dot(a, b[:, l * LW:(l + 1) * LW]) for l in range(b.shape[1] // LW)], axis=1)
            else:
                z = _dot(a, b)
            n = fcum[st["fi"] + 1] - fcum[st["fi"]]
            st["fi"] += 1
            nr, nl = z.shape[0] // 8, z.shape[1] // LW
            ties = {}
            for pos, v in st["ties"]:
                ties.setdefault(min(pos, nr * nl - 1), []).append(v)
            st["ties"] = []
            blk = lambda pos: z[8 * (pos % nr):8 * (pos % nr) + 8, (pos // nr) * LW:(pos // nr + 1) * LW]
            for u in range(n):
                pos = u * nr * nl // n
                v = vpu_unit(blk(pos))
                if pos + FD < nr * nl:
                    ties.setdefault(pos + FD, []).append(v)
                else:
                    st["ties"].append((pos + FD - nr * nl, v))
            if not ties:
                return z
            cols = []
            for l in range(nl):
                parts, r0 = [], 0
                for pos in sorted(p for p in ties if p // nr == l):
                    r = pos % nr
                    if r > r0:
                        parts.append(z[8 * r0:8 * r, l * LW:(l + 1) * LW])
                    zb = blk(pos)
                    for v in ties[pos]:
                        zb = jnp.maximum(zb, v)
                    parts.append(zb)
                    r0 = r + 1
                if r0 < nr:
                    parts.append(z[8 * r0:, l * LW:(l + 1) * LW])
                cols.append(jnp.concatenate(parts, axis=0))
            return jnp.concatenate(cols, axis=1)

        def wo_part(cg, r):
            rows = pl.ds(r * UR, UR)
            hp = (xT_s[rows, pl.ds(pl.multiple_of(col0 + cg * LW, LW), LW)].astype(F32)
                  + _dot(_up(woT_s[_h(r * UR, UR), pl.ds(0, KP)]), _up(oT_s[_h(0, KP), pl.ds(cg * LW, LW)])))
            hp_s[cg][rows, :] = hp
            st["c", cg] = _fold(hp) if r == 0 else st["c", cg] + _fold(hp)

        def wo_last_ln2(cg):
            lc = pl.ds(cg * LW, LW)
            ol = _up(oT_s[_h(KP, H * HP - KP), lc])
            shift = jnp.sum(st["c", cg], axis=0, keepdims=True) * (1.0 / D)
            p1, p2 = [], []
            for r in range(4):
                hr = (hp_s[cg][pl.ds(dz[0] + r * GW, GW), :]
                      + _dot(_up(woT_s[_h(r * GW, GW), pl.ds(KP, H * HP - KP)]), ol))
                h_s[cg][pl.ds(r * GW, GW), :] = hr
                d = hr - shift
                p1.append(_fold(d))
                p2.append(_fold(d * d))
            dm = _colmean(p1)
            rs = lax.rsqrt(jnp.maximum(_colmean(p2) - dm * dm, 0.0) + EPS)
            mu = shift + dm
            for r in range(4):
                hn_s[_h(r * GW, GW), lc] = _pk(((h_s[cg][pl.ds(dz[2] + r * GW, GW), :] - mu) * rs).astype(BF16))

        def ffn1(f0, fn, cg=None):
            hn = hn_s[...] if cg is None else hn_s[:, pl.ds(cg * LW, LW)]
            a = jnp.maximum(fdot(_up(w1T_s[_h(f0, fn), :]), _up(hn)), 0.0)
            return a * a

        queue = [(cg, r) for cg in range(NG) for r in range(D // UR)]

        def fill(n):
            for _ in range(min(n, len(queue))):
                wo_part(*queue.pop(0))

        for a in range(NI * NC + LAG):
            b = a - NC - LAG
            if b >= 0:
                probs_pv(b // NC, (b + ROT) % NC * CK, CK, 0, TQ, b % NC == 0, b % NC == NC - 1)
            if a < NI * NC:
                scores(a)
            else:
                fill(1)
        nch = NC // NG
        for cg in range(NG):
            for c in range(nch):
                if cg > 0 and c == T1:
                    assert all(q[0] >= cg for q in queue)
                    wo_last_ln2(cg - 1)
                probs_pv(NI - 1, (c + ROT // NG) % nch * CK * NG, CK * NG, cg * LW, LW, c == 0, c == nch - 1)
                fill(FILL[cg * nch + c])
        fill(len(queue))
        f0, fn = FCH[0]
        a00 = ffn1(f0, T2, 0)
        wo_last_ln2(NG - 1)
        a01 = ffn1(f0 + T2, fn - T2, 0)
        a_next = jnp.concatenate([jnp.concatenate([a00, a01], axis=0), ffn1(f0, fn, 1)], axis=1)

        load_q(nxt, a_next[fn - 1:, :])
        b2c = b2c_s[...]
        acc = jnp.concatenate([h_s[cg][pl.ds(dz[0], D), :] + b2c for cg in range(NG)], axis=1)
        for i, (f0, fn) in enumerate(FCH):
            a = a_next.astype(BF16)
            if i < len(FCH) - 1:
                a_next = ffn1(*FCH[i + 1])
                acc = acc + fdot(w2T_s[:, pl.ds(f0, fn)], a)
            else:
                for og in range(D // OR):
                    res = acc[og * OR:(og + 1) * OR, :] + fdot(w2T_s[pl.ds(og * OR, OR), pl.ds(f0, fn)], a)
                    out_s[t, pl.ds(og * OR, OR), :] = res.astype(BF16)
                    out_copy(t, og).start()
        assert not units

    def step(i, carry):
        pl.when(i == 0)(prologue)
        pl.when(i > 0)(lambda: tile(i - 1))
        return carry

    lax.fori_loop(0, NT + 1, step, 0)
    for t in range(NT):
        for og in range(D // OR):
            out_copy(t, og).wait()


@jax.jit
def pallas_sequential_preLN__mha_block__dense_activation_squared_relu__prompt_kernel(
    A_x: jax.Array,
    A_wqkv: jax.Array,
    A_wo: jax.Array,
    B_x: jax.Array,
    B_w1: jax.Array,
    B_b1: jax.Array,
    B_w2: jax.Array,
    B_b2: jax.Array,
):
    del B_x
    hbm = pl.BlockSpec(memory_space=pltpu.HBM)
    outT = pl.pallas_call(
        _kernel,
        out_shape=jax.ShapeDtypeStruct((1, D, S), BF16),
        in_specs=[hbm] * 7,
        out_specs=hbm,
        scratch_shapes=[
            pltpu.VMEM((D, S), BF16),
            pltpu.VMEM((D, 3 * D), BF16),
            pltpu.VMEM((D, D), BF16),
            pltpu.VMEM((DA, F), BF16),
            pltpu.VMEM((F,), BF16),
            pltpu.VMEM((D, F), BF16),
            pltpu.VMEM((D,), BF16),
            pltpu.VMEM((3 * D // 2, D), U32),
            pltpu.VMEM((D // 2, H * HP), U32),
            pltpu.VMEM((F // 2, DA), U32),
            pltpu.VMEM((D, LW), F32),
            pltpu.VMEM((D // 2, S), U32),
            pltpu.VMEM((4, S // 2, 128), U32),
            pltpu.VMEM((D, NV, 128), F32),
            pltpu.VMEM((DA // 2, S), U32),
            pltpu.VMEM((DA // 2, TQ), U32),
            pltpu.VMEM((D, TQ), F32),
            pltpu.VMEM((D, TQ), F32),
            pltpu.VMEM((H * HP // 2, S), U32),
            pltpu.VMEM((S, SW), F32),
            pltpu.VMEM((S, SW), F32),
            pltpu.VMEM((S, SW), F32),
            pltpu.VMEM((NI, NV, SW), F32),
            pltpu.VMEM((H * HP // 2, TQ), U32),
            pltpu.VMEM((DA // 2, TQ), U32),
            pltpu.VMEM((NT, D, TQ), BF16),
            pltpu.SMEM((3,), jnp.int32),
            pltpu.SMEM((3,), jnp.int32),
            pltpu.SemaphoreType.DMA((6,)),
        ] + [pltpu.VMEM((D, LW), F32)] * (2 * NG),
        compiler_params=pltpu.CompilerParams(vmem_limit_bytes=100 * 1024 * 1024,
                                             disable_bounds_checks=True,
                                             disable_semaphore_checks=True),
        name="fused_block",
    )(jnp.transpose(A_x, (0, 2, 1)), A_wqkv, A_wo, B_w1, B_b1, B_w2.T, B_b2)
    return jnp.transpose(outT, (0, 2, 1))
```

```python
import jax
import jax.numpy as jnp
from jax import lax
import jax.experimental.pallas as pl
import jax.experimental.pallas.tpu as pltpu

S, D, H, DH, F = 2048, 448, 16, 28, 1792
HP = 32
GW = 4 * DH
DA = 464
PC = 512
TQ = 256
NT = S // TQ
HPI = 2
NI = H // HPI
SW = HPI * TQ
CK = 128
NC = S // CK
LAG = 3
LW = 128
NG = TQ // LW
NLT = SW // LW
KP = 3 * 128
UR = 64
FCH = ((0, 512), (512, 512), (1024, 512), (1536, 256))
OR = 224
FILL = (0, 1, 0, 1, 1, 1, 0, 0, 1, 1, 1, 0, 0, 1, 0, 1)
T1, T2, ROT = 5, 160, 2
W0, W1, XA = 384, 640, 256
KA, KS, VS = 576, 720, 384
TB1, TB2 = 23, 160
NV, UK = 192, 16
NKG = NV // UK
NCH = NLT * NKG
RP = (2, 1, 2, 2, 3, 1, 2, 2, 3, 2, 2, 2, 2, 2, 2, 2)
RATE = [2 if a < NC + LAG else (RP[a % NC] if a < NI * NC - 4 else 0) for a in range(NI * NC)]
NA = NI * NCH - sum(RATE)
PA, PL = -(-NA // NCH), NA // NCH
QLO, QHI = -(-PA * HPI * DH // 16) * 16, PL * HPI * DH // 16 * 16
FW = (0, 0.7, 1, 1, 1.15, 1, 1, 1, 1, 0.5, 0)
TD, FD = 2, 32
MCH = [NV + 16 * (c * ((S - NV) // 16) // NC) for c in range(NC + 1)]
EPS = 1e-5
QSCALE = (DH ** -0.5) * 1.4426950408889634
LOWEST = -3.0e38
F32 = jnp.float32
BF16 = jnp.bfloat16
U32 = jnp.uint32


def _pad_heads_rows(m, filler):
    parts = []
    for h in range(H):
        parts.append(m[DH * h:DH * (h + 1), :])
        parts.append(filler)
    return jnp.concatenate(parts, axis=0)


def _fold(v):
    v = jnp.sum(v.reshape(v.shape[0] // 16, 16, v.shape[1]), axis=0)
    return v[:8] + v[8:]


def _colmean(parts):
    return jnp.sum((parts[0] + parts[1]) + (parts[2] + parts[3]), axis=0, keepdims=True) * (1.0 / D)


def _pk(x):
    return pltpu.bitcast(x, U32)


def _up(x):
    return pltpu.bitcast(x, BF16)


def _h(start, size):
    return pl.ds(start // 2, size // 2)


def _dot(a, b):
    return jnp.dot(a, b, preferred_element_type=F32)


def _unit(u):
    return u % NLT, (u // NLT + 4 * (u % NLT)) % NKG


def _kernel(xT_hbm, wqkv_hbm, wo_hbm, w1_hbm, b1_hbm, w2T_hbm, b2_hbm, out_hbm,
            xT_s, wqkv_s, wo_s, w1_s, b1_s, w2T_s, b2_s,
            wT_s, woT_s, w1T_s, b2c_s, xn_s,
            k_s, kb_s, qT_s, qc_s, qf_s, qn_s, vT_s, s0, s1, s2, sv_s, oT_s, hn_s, out_s,
            zero_s, dz_s, sems, *hbufs):
    def w_copy(c0, n, sem):
        return pltpu.make_async_copy(wqkv_hbm.at[:, pl.ds(c0, n)], wqkv_s.at[:, pl.ds(c0, n)], sems.at[sem])

    def x_copy(c0, n, sem):
        return [pltpu.make_async_copy(xT_hbm.at[0, :, pl.ds(c, TQ)], xT_s.at[c // TQ], sems.at[sem])
                for c in range(c0, c0 + n, TQ)]

    grp_a = [w_copy(W0, W1 - W0, 0)] + x_copy(0, XA, 0)
    grp_b = x_copy(XA, PC - XA, 1) + [w_copy(W1, 2 * D - W1, 1)]
    grp_c = [w_copy(0, W0, 3)]
    grp_d = [w_copy(2 * D, D, 2)] + x_copy(PC, PC, 2)
    grp_e = x_copy(2 * PC, 2 * PC, 4) + [
             pltpu.make_async_copy(wo_hbm, wo_s, sems.at[4]),
             pltpu.make_async_copy(w1_hbm, w1_s.at[pl.ds(0, D), :], sems.at[4]),
             pltpu.make_async_copy(b1_hbm, b1_s, sems.at[4]),
             pltpu.make_async_copy(b2_hbm, b2_s, sems.at[4])]
    grp_f = [pltpu.make_async_copy(w2T_hbm, w2T_s, sems.at[0])]

    def start(grp):
        for cp in grp:
            cp.start()

    def wait(grp):
        for cp in grp:
            cp.wait()

    start(grp_a)
    start(grp_b)
    for k in range(3):
        zero_s[k] = 0
        dz_s[k] = 0
    zeros0 = [pl.multiple_of(zero_s[k], 16) for k in range(3)]
    zero = zeros0[0]
    qT_s[:, _h(D, DA - D), :] = jnp.zeros((NT, (DA - D) // 2, TQ), U32)
    arow = lax.broadcasted_iota(jnp.int32, (DA - D, TQ), 0)
    hn_s[_h(D, DA - D), :] = _pk(jnp.where(arow == 0, 1.0, 0.0).astype(BF16))

    def ln1(c0, c1, split=False):
        zeros = zeros0 if split else [pl.multiple_of(dz_s[k], 16) for k in range(3)]
        for cg in range(c0 // LW, c1 // LW):
            cols = pl.ds(cg * LW, LW)
            xt, xc = cg // NG, pl.ds(cg % NG * LW, LW)
            if split:
                ld = lambda k, r: xT_s[xt, pl.ds(zeros[k] + r * GW, GW), xc].astype(F32)
                mu = _colmean([_fold(ld(0, r)) for r in range(4)])
                var = _colmean([_fold(jnp.square(ld(1, r) - mu)) for r in range(4)])
                rs = lax.rsqrt(var + EPS)
                for r in range(4):
                    xn_s[_h(r * GW, GW), cols] = _pk(((ld(2, r) - mu) * rs).astype(BF16))
            else:
                ld = lambda k: xT_s[xt, pl.ds(zeros[k], D), xc].astype(F32)
                mu = jnp.sum(ld(0), axis=0, keepdims=True) * (1.0 / D)
                var = jnp.sum(jnp.square(ld(1) - mu), axis=0, keepdims=True) * (1.0 / D)
                xn_s[:, cols] = _pk(((ld(2) - mu) * lax.rsqrt(var + EPS)).astype(BF16))

    def w_transpose(c0, n):
        wT_s[_h(c0, n), :] = _pk(wqkv_s[:, pl.ds(c0, n)].T)

    def k_table(d0, d1, gate=None):
        for g in range(4):
            lo, hi = max(d0, g * GW), min(d1, (g + 1) * GW)
            if lo >= hi:
                continue
            kp = k_s[g, pl.ds(zero, NV // 2), :]
            if gate is not None:
                kp = kp | pltpu.bitcast(gate - gate, U32)
            kb_s[pl.ds(lo, hi - lo)] = jnp.concatenate(
                [_up(jnp.broadcast_to(kp[:, d - g * GW:d - g * GW + 1], (NV // 2, 128))).astype(F32)[None]
                 for d in range(lo, hi)], axis=0)

    def proj(r0, r1, c0, c1):
        xr = pl.ds(zero if c0 >= PC else 0, D // 2)
        return _dot(_up(wT_s[_h(r0, r1 - r0), :]), _up(xn_s[xr, pl.ds(c0, c1 - c0)]))

    def put_q(z, r0, c0):
        c = c0
        while c < c0 + z.shape[1]:
            n = min(TQ - c % TQ, c0 + z.shape[1] - c)
            qT_s[c // TQ, _h(r0, z.shape[0]), pl.ds(c % TQ, n)] = _pk((z[:, c - c0:c - c0 + n] * QSCALE).astype(BF16))
            c += n

    def put_k(kT, c0):
        for g in range(4):
            k_s[g, _h(c0, kT.shape[1]), :] = _pk(kT[GW * g:GW * g + 128, :].astype(BF16).T)

    def put_v(vT, c0):
        ones_row = jnp.where(lax.broadcasted_iota(jnp.int32, (HP - DH, PC), 0) == 0, 1.0, 0.0)
        vT_s[:, pl.ds(c0, PC)] = _pk(_pad_heads_rows(vT, ones_row).astype(BF16))

    def proj_q(r0, r1, c0, c1):
        put_q(proj(r0, r1, c0, c1), r0, c0)

    def proj_kv(c0):
        kv = proj(D, 3 * D, c0, c0 + PC)
        put_k(kv, c0)
        put_v(kv[D:, :], c0)

    def load_q(tq, gate=None):
        q = qT_s[tq, _h(0, DA), :]
        qc_s[...] = q
        qf = _up(q[QHI // 2:D // 2]).astype(F32)
        if gate is not None:
            qf = qf + (gate - gate)
        qf_s[pl.ds(QHI, D - QHI), :] = qf

    qrow = lax.broadcasted_iota(jnp.int32, (128, TQ), 0)

    def qweights(i):
        q = _up(qc_s[_h((i * HPI) // 4 * GW, 128), :]).astype(F32)
        js = [(i * HPI + k) % 4 for k in range(HPI)]
        return jnp.concatenate(
            [jnp.where((qrow >= DH * j) & (qrow < DH * (j + 1)), q, 0.0) for j in js], axis=1).astype(BF16)

    def prologue():
        pk = lambda r0, r1, c0, c1: proj(r0, r1, c0, c1).astype(BF16)
        pad = lambda n: jnp.zeros((DA - D, n), BF16)
        wait(grp_a)
        start(grp_c)
        start(grp_d)
        for c0 in range(W0, W1, 128):
            w_transpose(c0, 128)
        ln1(0, XA, True)
        proj_q(W0, D, 0, XA)
        k1 = pk(D, KA, 0, XA)
        wait(grp_b)
        for c0 in range(W1, 2 * D, 128):
            w_transpose(c0, 128)
        ln1(XA, XA + LW, True)
        k2 = pk(KA, W1, 0, XA)
        ln1(XA + LW, PC)
        put_k(jnp.concatenate([k1, k2, pk(W1, 2 * D, 0, XA), pad(XA)], axis=0), 0)
        k3 = pk(D, KS, XA, PC)
        wait(grp_c)
        start(grp_e)
        w_transpose(0, W0)
        k_table(0, TB1)
        put_k(jnp.concatenate([k3, pk(KS, 2 * D, XA, PC), pad(PC - XA)], axis=0), XA)
        proj_q(W0, D, XA, PC)
        proj_q(0, W0, 0, VS)
        wait(grp_d)
        start(grp_f)
        w_transpose(2 * D, D)
        proj_q(0, W0, VS, PC)
        k_table(TB1, TB2)
        ln1(PC, 2 * PC)
        put_v(proj(2 * D, 3 * D, 0, PC), 0)
        proj_kv(PC)
        wait(grp_e)
        ln1(2 * PC, 3 * PC)
        z = proj(0, D, PC, 2 * PC)
        k_table(TB2, D, z[0:1, 0:LW])
        put_q(z, 0, PC)
        ln1(3 * PC, 4 * PC)
        proj_kv(2 * PC)
        proj_q(0, D, 2 * PC, 3 * PC)
        proj_kv(3 * PC)
        proj_q(0, D, 3 * PC, 4 * PC)
        woT_s[...] = _pk(_pad_heads_rows(wo_s[...].astype(F32), jnp.zeros((HP - DH, D), F32)).astype(BF16).T)
        brow = lax.broadcasted_iota(jnp.int32, (DA - D, F), 0)
        w1_s[pl.ds(D, DA - D), :] = jnp.where(brow == 0, b1_s[...].astype(F32).reshape(1, F), 0.0).astype(BF16)
        w1T_s[...] = _pk(w1_s[...].T)
        b2c_s[...] = jnp.broadcast_to(b2_s[...].astype(F32).reshape(1, D), (LW, D)).T
        load_q(0)
        for i in range(PA):
            sv_s[i] = _dot(_up(k_s[(i * HPI) // 4, _h(0, NV), :]), qweights(i))
        wait(grp_f)

    bufs = (s0, s1, s2)
    h_s, hp_s = hbufs[:NG], hbufs[NG:]

    def out_copy(t, og):
        return pltpu.make_async_copy(out_s.at[t, pl.ds(og * OR, OR), :],
                                     out_hbm.at[0, pl.ds(og * OR, OR), pl.ds(pl.multiple_of(t * TQ, TQ), TQ)],
                                     sems.at[5])

    def tile(t):
        dz = [pl.multiple_of(dz_s[k], 16) for k in range(3)]
        st = {"m": {}, "pend": [], "ties": [], "fi": 0}

        nxt = jnp.minimum(t + 1, NT - 1)
        qn_s[pl.ds(zero, QLO), :] = _up(qT_s[nxt, _h(0, QLO), :]).astype(F32)
        units = [(i,) + _unit(u) + (i * NCH + u < NA,) for i in range(NI) for u in range(NCH)]
        units = units[NA:] + units[:NA]

        def vpu_unit(gate):
            i, lt, kg, ahead = units.pop(0)
            h = i * HPI + lt // NG
            if ("qv", i, lt, ahead) not in st:
                q_ref = qn_s if ahead else qf_s
                st["qv", i, lt, ahead] = jnp.concatenate(
                    [jnp.broadcast_to(q_ref[pl.ds(h * DH + d, 1), pl.ds(lt % NG * LW, LW)], (UK, LW))[None]
                     for d in range(DH)], axis=0)
            prod = kb_s[pl.ds(h * DH, DH), pl.ds(kg * UK, UK), :] * st["qv", i, lt, ahead]
            z0 = jnp.concatenate([gate - gate] * (UK // 8), axis=0)
            acc = jnp.sum(jnp.concatenate([z0[None], prod], axis=0), axis=0)
            sv_s[i, pl.ds(kg * UK, UK), pl.ds(lt * LW, LW)] = acc
            return jnp.minimum(jnp.min(acc.reshape(UK // 8, 8, LW), axis=0), LOWEST)

        def scores(a):
            i, c = a // NC, a % NC
            if c == 0:
                st["qm"] = qweights(i)
            k0, nk = MCH[c], MCH[c + 1] - MCH[c]
            s = _dot(_up(k_s[(i * HPI) // 4, _h(k0, nk), :]), st["qm"])
            bufs[i % 3][pl.ds(k0, nk), :] = s
            for lt in range(NLT):
                m = jnp.max(s[:, lt * LW:(lt + 1) * LW].reshape(nk // 8, 8, LW), axis=0)
                st["m8", lt] = m if c == 0 else jnp.maximum(m, st["m8", lt])
            pend = st["pend"]
            for j in range(RATE[a]):
                r, lt = j * (nk // 8) // RATE[a] + 1, 2 * j % NLT
                pend.append((a + TD, (lt + 2) % NLT, vpu_unit(s[8 * r:8 * r + 8, lt * LW:(lt + 1) * LW])))
            while pend and pend[0][0] <= a:
                _, lt, v = pend.pop(0)
                st["m8", lt] = jnp.maximum(st["m8", lt], v)
            for u in range(c * NCH // NC, (c + 1) * NCH // NC):
                lt, kg = _unit(u)
                assert (i, lt, kg, False) not in units
                sv = sv_s[i, pl.ds(zero + kg * UK, UK), pl.ds(lt * LW, LW)]
                st["m8", lt] = jnp.maximum(st["m8", lt], jnp.max(sv.reshape(UK // 8, 8, LW), axis=0))
            if c == NC - 1:
                m8 = jnp.concatenate([st["m8", lt] for lt in range(NLT)], axis=1)
                st["m"][i] = jnp.max(m8, axis=0, keepdims=True)

        def probs_pv(i, k0, nk, q0, nq, first, last):
            for k in range(HPI):
                h = i * HPI + k
                lo = k * TQ + q0
                parts = []
                if k0 < NV:
                    parts.append(sv_s[i, pl.ds(zero + k0, min(NV - k0, nk)), pl.ds(lo, nq)])
                if k0 + nk > NV:
                    parts.append(bufs[i % 3][pl.ds(zero + max(k0, NV), k0 + nk - max(k0, NV)), pl.ds(lo, nq)])
                p = jnp.exp2(jnp.concatenate(parts, axis=0) - st["m"][i][:, lo:lo + nq])
                pv = _dot(_up(vT_s[_h(h * HP, HP), pl.ds(k0, nk)]), p.astype(BF16))
                acc = pv if first else st["acc", k] + pv
                st["acc", k] = acc
                if last:
                    l = acc[DH:DH + 1, :]
                    r = pl.reciprocal(l, approx=True)
                    r = r * (2.0 - l * r)
                    oT_s[_h(h * HP, HP), pl.ds(q0, nq)] = _pk((acc * r).astype(BF16))

        fcost = [T2, FCH[0][1] - T2, FCH[0][1]]
        for idx, (f0, fn) in enumerate(FCH):
            if idx < len(FCH) - 1:
                fcost += [2 * FCH[idx + 1][1], D * fn // 256]
            else:
                fcost += [OR * fn // 256] * (D // OR)
        fcost = [c * w for c, w in zip(fcost, FW)]
        fcum = [int(sum(fcost[:j]) * NA / sum(fcost) + 1e-6) for j in range(len(fcost) + 1)]

        def fdot(a, b):
            if b.shape[0] > 256 and b.shape[1] > LW:
                z = jnp.concatenate([_dot(a, b[:, l * LW:(l + 1) * LW]) for l in range(b.shape[1] // LW)], axis=1)
            else:
                z = _dot(a, b)
            n = fcum[st["fi"] + 1] - fcum[st["fi"]]
            st["fi"] += 1
            nr, nl = z.shape[0] // 8, z.shape[1] // LW
            ties = {}
            for pos, v in st["ties"]:
                ties.setdefault(min(pos, nr * nl - 1), []).append(v)
            st["ties"] = []
            blk = lambda pos: z[8 * (pos % nr):8 * (pos % nr) + 8, (pos // nr) * LW:(pos // nr + 1) * LW]
            for u in range(n):
                pos = u * nr * nl // n
                v = vpu_unit(blk(pos))
                if pos + FD < nr * nl:
                    ties.setdefault(pos + FD, []).append(v)
                else:
                    st["ties"].append((pos + FD - nr * nl, v))
            if not ties:
                return z
            cols = []
            for l in range(nl):
                parts, r0 = [], 0
                for pos in sorted(p for p in ties if p // nr == l):
                    r = pos % nr
                    if r > r0:
                        parts.append(z[8 * r0:8 * r, l * LW:(l + 1) * LW])
                    zb = blk(pos)
                    for v in ties[pos]:
                        zb = jnp.maximum(zb, v)
                    parts.append(zb)
                    r0 = r + 1
                if r0 < nr:
                    parts.append(z[8 * r0:, l * LW:(l + 1) * LW])
                cols.append(jnp.concatenate(parts, axis=0))
            return jnp.concatenate(cols, axis=1)

        def wo_part(cg, r):
            rows = pl.ds(r * UR, UR)
            hp = (xT_s[t, rows, pl.ds(cg * LW, LW)].astype(F32)
                  + _dot(_up(woT_s[_h(r * UR, UR), pl.ds(0, KP)]), _up(oT_s[_h(0, KP), pl.ds(cg * LW, LW)])))
            hp_s[cg][rows, :] = hp
            st["c", cg] = _fold(hp) if r == 0 else st["c", cg] + _fold(hp)

        def wo_last_ln2(cg):
            lc = pl.ds(cg * LW, LW)
            ol = _up(oT_s[_h(KP, H * HP - KP), lc])
            shift = jnp.sum(st["c", cg], axis=0, keepdims=True) * (1.0 / D)
            p1, p2 = [], []
            for r in range(4):
                hr = (hp_s[cg][pl.ds(dz[0] + r * GW, GW), :]
                      + _dot(_up(woT_s[_h(r * GW, GW), pl.ds(KP, H * HP - KP)]), ol))
                h_s[cg][pl.ds(r * GW, GW), :] = hr
                d = hr - shift
                p1.append(_fold(d))
                p2.append(_fold(d * d))
            dm = _colmean(p1)
            rs = lax.rsqrt(jnp.maximum(_colmean(p2) - dm * dm, 0.0) + EPS)
            mu = shift + dm
            for r in range(4):
                hn_s[_h(r * GW, GW), lc] = _pk(((h_s[cg][pl.ds(dz[2] + r * GW, GW), :] - mu) * rs).astype(BF16))

        def ffn1(f0, fn, cg=None):
            hn = hn_s[...] if cg is None else hn_s[:, pl.ds(cg * LW, LW)]
            a = jnp.maximum(fdot(_up(w1T_s[_h(f0, fn), :]), _up(hn)), 0.0)
            return a * a

        queue = [(cg, r) for cg in range(NG) for r in range(D // UR)]

        def fill(n):
            for _ in range(min(n, len(queue))):
                wo_part(*queue.pop(0))

        for a in range(NI * NC + LAG):
            b = a - NC - LAG
            if b >= 0:
                probs_pv(b // NC, (b + ROT) % NC * CK, CK, 0, TQ, b % NC == 0, b % NC == NC - 1)
            if a < NI * NC:
                scores(a)
            else:
                fill(1)
        nch = NC // NG
        for cg in range(NG):
            for c in range(nch):
                if cg > 0 and c == T1:
                    assert all(q[0] >= cg for q in queue)
                    wo_last_ln2(cg - 1)
                probs_pv(NI - 1, (c + ROT // NG) % nch * CK * NG, CK * NG, cg * LW, LW, c == 0, c == nch - 1)
                fill(FILL[cg * nch + c])
        fill(len(queue))
        f0, fn = FCH[0]
        a00 = ffn1(f0, T2, 0)
        wo_last_ln2(NG - 1)
        a01 = ffn1(f0 + T2, fn - T2, 0)
        a_next = jnp.concatenate([jnp.concatenate([a00, a01], axis=0), ffn1(f0, fn, 1)], axis=1)

        load_q(nxt, a_next[fn - 1:, :])
        b2c = b2c_s[...]
        acc = jnp.concatenate([h_s[cg][pl.ds(dz[0], D), :] + b2c for cg in range(NG)], axis=1)
        for i, (f0, fn) in enumerate(FCH):
            a = a_next.astype(BF16)
            if i < len(FCH) - 1:
                a_next = ffn1(*FCH[i + 1])
                acc = acc + fdot(w2T_s[:, pl.ds(f0, fn)], a)
            else:
                for og in range(D // OR):
                    res = acc[og * OR:(og + 1) * OR, :] + fdot(w2T_s[pl.ds(og * OR, OR), pl.ds(f0, fn)], a)
                    out_s[t, pl.ds(og * OR, OR), :] = res.astype(BF16)
                    out_copy(t, og).start()
        assert not units

    def step(i, carry):
        pl.when(i == 0)(prologue)
        pl.when(i > 0)(lambda: tile(i - 1))
        return carry

    lax.fori_loop(0, NT + 1, step, 0)
    for t in range(NT):
        for og in range(D // OR):
            out_copy(t, og).wait()


@jax.jit
def pallas_sequential_preLN__mha_block__dense_activation_squared_relu__prompt_kernel(
    A_x: jax.Array,
    A_wqkv: jax.Array,
    A_wo: jax.Array,
    B_x: jax.Array,
    B_w1: jax.Array,
    B_b1: jax.Array,
    B_w2: jax.Array,
    B_b2: jax.Array,
):
    del B_x
    hbm = pl.BlockSpec(memory_space=pltpu.HBM)
    outT = pl.pallas_call(
        _kernel,
        out_shape=jax.ShapeDtypeStruct((1, D, S), BF16),
        in_specs=[hbm] * 7,
        out_specs=hbm,
        scratch_shapes=[
            pltpu.VMEM((NT, D, TQ), BF16),
            pltpu.VMEM((D, 3 * D), BF16),
            pltpu.VMEM((D, D), BF16),
            pltpu.VMEM((DA, F), BF16),
            pltpu.VMEM((F,), BF16),
            pltpu.VMEM((D, F), BF16),
            pltpu.VMEM((D,), BF16),
            pltpu.VMEM((3 * D // 2, D), U32),
            pltpu.VMEM((D // 2, H * HP), U32),
            pltpu.VMEM((F // 2, DA), U32),
            pltpu.VMEM((D, LW), F32),
            pltpu.VMEM((D // 2, S), U32),
            pltpu.VMEM((4, S // 2, 128), U32),
            pltpu.VMEM((D, NV, 128), F32),
            pltpu.VMEM((NT, 256, TQ), U32),
            pltpu.VMEM((DA // 2, TQ), U32),
            pltpu.VMEM((D, TQ), F32),
            pltpu.VMEM((D, TQ), F32),
            pltpu.VMEM((H * HP // 2, S), U32),
            pltpu.VMEM((S, SW), F32),
            pltpu.VMEM((S, SW), F32),
            pltpu.VMEM((S, SW), F32),
            pltpu.VMEM((NI, NV, SW), F32),
            pltpu.VMEM((H * HP // 2, TQ), U32),
            pltpu.VMEM((DA // 2, TQ), U32),
            pltpu.VMEM((NT, D, TQ), BF16),
            pltpu.SMEM((3,), jnp.int32),
            pltpu.SMEM((3,), jnp.int32),
            pltpu.SemaphoreType.DMA((6,)),
        ] + [pltpu.VMEM((D, LW), F32)] * (2 * NG),
        compiler_params=pltpu.CompilerParams(vmem_limit_bytes=100 * 1024 * 1024,
                                             disable_bounds_checks=True,
                                             disable_semaphore_checks=True),
        name="fused_block",
    )(jnp.transpose(A_x, (0, 2, 1)), A_wqkv, A_wo, B_w1, B_b1, B_w2.T, B_b2)
    return jnp.transpose(outT, (0, 2, 1))
```

```python
import jax
import jax.numpy as jnp
from jax import lax
import jax.experimental.pallas as pl
import jax.experimental.pallas.tpu as pltpu

S, D, H, DH, F = 2048, 448, 16, 28, 1792
HP = 32
GW = 4 * DH
DA = 464
PC = 512
TQ = 256
NT = S // TQ
HPI = 2
NI = H // HPI
SW = HPI * TQ
CK = 128
NC = S // CK
LAG = 3
LW = 128
NG = TQ // LW
NLT = SW // LW
KP = 3 * 128
UR = 64
FCH = ((0, 512), (512, 512), (1024, 512), (1536, 256))
OR = 224
FILL = (0, 1, 0, 1, 1, 1, 0, 0, 1, 1, 1, 0, 0, 1, 0, 1)
T1, T2, ROT = 5, 160, 4
W0, W1, XA = 384, 640, 256
KA, KS, VS = 576, 720, 384
TB1, TB2 = 23, 160
NV, UK = 192, 16
NKG = NV // UK
NCH = NLT * NKG
RA = (2, 2, 2, 2, 2, 3, 3) + (2,) * 12
RP = (2, 1, 2, 2, 3, 1, 2, 2, 3, 1, 2, 2, 2, 2, 2, 2)
RATE = [RA[a] if a < NC + LAG else (RP[a % NC] if a < NI * NC - 4 else 0) for a in range(NI * NC)]
GATE = {1: ((8, 0),), 2: ((1, 0), (7, 2)), 3: ((1, 0), (5, 2), (10, 2))}
NA = NI * NCH - sum(RATE)
PA, PL = -(-NA // NCH), NA // NCH
QLO, QHI = -(-PA * HPI * DH // 16) * 16, PL * HPI * DH // 16 * 16
FW = (0, 0.7, 1, 1, 1.15, 1, 1, 1, 1, 0.5, 0.15)
TD, FD = 2, 32
MCH = [NV + 16 * (c * ((S - NV) // 16) // NC) for c in range(NC + 1)]
EPS = 1e-5
QSCALE = (DH ** -0.5) * 1.4426950408889634
LOWEST = -3.0e38
F32 = jnp.float32
BF16 = jnp.bfloat16
U32 = jnp.uint32


def _pad_heads_rows(m, filler):
    parts = []
    for h in range(H):
        parts.append(m[DH * h:DH * (h + 1), :])
        parts.append(filler)
    return jnp.concatenate(parts, axis=0)


def _fold(v):
    v = jnp.sum(v.reshape(v.shape[0] // 16, 16, v.shape[1]), axis=0)
    return v[:8] + v[8:]


def _colmean(parts):
    return jnp.sum((parts[0] + parts[1]) + (parts[2] + parts[3]), axis=0, keepdims=True) * (1.0 / D)


def _pk(x):
    return pltpu.bitcast(x, U32)


def _up(x):
    return pltpu.bitcast(x, BF16)


def _h(start, size):
    return pl.ds(start // 2, size // 2)


def _dot(a, b):
    return jnp.dot(a, b, preferred_element_type=F32)


def _unit(u):
    return u % NLT, (u // NLT + 5 * (u % NLT)) % NKG


def _kernel(xT_hbm, wqkv_hbm, wo_hbm, w1_hbm, b1_hbm, w2T_hbm, b2_hbm, out_hbm,
            xT_s, wqkv_s, wo_s, w1_s, b1_s, w2T_s, b2_s,
            wT_s, woT_s, w1T_s, b2c_s, xn_s,
            k_s, kb_s, qT_s, qc_s, qf_s, qn_s, vT_s, s0, s1, s2, sv_s, oT_s, hn_s, out_s,
            zero_s, dz_s, sems, *hbufs):
    def w_copy(c0, n, sem):
        return pltpu.make_async_copy(wqkv_hbm.at[:, pl.ds(c0, n)], wqkv_s.at[:, pl.ds(c0, n)], sems.at[sem])

    def x_copy(c0, n, sem):
        return [pltpu.make_async_copy(xT_hbm.at[0, :, pl.ds(c, TQ)], xT_s.at[c // TQ], sems.at[sem])
                for c in range(c0, c0 + n, TQ)]

    grp_a = [w_copy(W0, W1 - W0, 0)] + x_copy(0, XA, 0)
    grp_b = x_copy(XA, PC - XA, 1) + [w_copy(W1, 2 * D - W1, 1)]
    grp_c = [w_copy(0, W0, 3)]
    grp_d = [w_copy(2 * D, D, 2)] + x_copy(PC, PC, 2)
    grp_e = x_copy(2 * PC, 2 * PC, 4) + [
             pltpu.make_async_copy(wo_hbm, wo_s, sems.at[4]),
             pltpu.make_async_copy(w1_hbm, w1_s.at[pl.ds(0, D), :], sems.at[4]),
             pltpu.make_async_copy(b1_hbm, b1_s, sems.at[4]),
             pltpu.make_async_copy(b2_hbm, b2_s, sems.at[4])]
    grp_f = [pltpu.make_async_copy(w2T_hbm, w2T_s, sems.at[0])]

    def start(grp):
        for cp in grp:
            cp.start()

    def wait(grp):
        for cp in grp:
            cp.wait()

    start(grp_a)
    start(grp_b)
    for k in range(3):
        zero_s[k] = 0
        dz_s[k] = 0
    zeros0 = [pl.multiple_of(zero_s[k], 16) for k in range(3)]
    zero = zeros0[0]
    qT_s[:, _h(D, DA - D), :] = jnp.zeros((NT, (DA - D) // 2, TQ), U32)
    arow = lax.broadcasted_iota(jnp.int32, (DA - D, TQ), 0)
    hn_s[_h(D, DA - D), :] = _pk(jnp.where(arow == 0, 1.0, 0.0).astype(BF16))

    def ln1(c0, c1, split=False):
        zeros = zeros0 if split else [pl.multiple_of(dz_s[k], 16) for k in range(3)]
        for cg in range(c0 // LW, c1 // LW):
            cols = pl.ds(cg * LW, LW)
            xt, xc = cg // NG, pl.ds(cg % NG * LW, LW)
            if split:
                ld = lambda k, r: xT_s[xt, pl.ds(zeros[k] + r * GW, GW), xc].astype(F32)
                mu = _colmean([_fold(ld(0, r)) for r in range(4)])
                var = _colmean([_fold(jnp.square(ld(1, r) - mu)) for r in range(4)])
                rs = lax.rsqrt(var + EPS)
                for r in range(4):
                    xn_s[_h(r * GW, GW), cols] = _pk(((ld(2, r) - mu) * rs).astype(BF16))
            else:
                ld = lambda k: xT_s[xt, pl.ds(zeros[k], D), xc].astype(F32)
                mu = jnp.sum(ld(0), axis=0, keepdims=True) * (1.0 / D)
                var = jnp.sum(jnp.square(ld(1) - mu), axis=0, keepdims=True) * (1.0 / D)
                xn_s[:, cols] = _pk(((ld(2) - mu) * lax.rsqrt(var + EPS)).astype(BF16))

    def w_transpose(c0, n):
        wT_s[_h(c0, n), :] = _pk(wqkv_s[:, pl.ds(c0, n)].T)

    def k_table(d0, d1, gate=None):
        for g in range(4):
            lo, hi = max(d0, g * GW), min(d1, (g + 1) * GW)
            if lo >= hi:
                continue
            kp = k_s[g, pl.ds(zero, NV // 2), :]
            if gate is not None:
                kp = kp | pltpu.bitcast(gate - gate, U32)
            kb_s[pl.ds(lo, hi - lo)] = jnp.concatenate(
                [_up(jnp.broadcast_to(kp[:, d - g * GW:d - g * GW + 1], (NV // 2, 128))).astype(F32)[None]
                 for d in range(lo, hi)], axis=0)

    def proj(r0, r1, c0, c1):
        xr = pl.ds(zero if c0 >= PC else 0, D // 2)
        return _dot(_up(wT_s[_h(r0, r1 - r0), :]), _up(xn_s[xr, pl.ds(c0, c1 - c0)]))

    def put_q(z, r0, c0):
        c = c0
        while c < c0 + z.shape[1]:
            n = min(TQ - c % TQ, c0 + z.shape[1] - c)
            qT_s[c // TQ, _h(r0, z.shape[0]), pl.ds(c % TQ, n)] = _pk((z[:, c - c0:c - c0 + n] * QSCALE).astype(BF16))
            c += n

    def put_k(kT, c0):
        for g in range(4):
            k_s[g, _h(c0, kT.shape[1]), :] = _pk(kT[GW * g:GW * g + 128, :].astype(BF16).T)

    def put_v(vT, c0):
        ones_row = jnp.where(lax.broadcasted_iota(jnp.int32, (HP - DH, PC), 0) == 0, 1.0, 0.0)
        vT_s[:, pl.ds(c0, PC)] = _pk(_pad_heads_rows(vT, ones_row).astype(BF16))

    def proj_q(r0, r1, c0, c1):
        put_q(proj(r0, r1, c0, c1), r0, c0)

    def proj_kv(c0):
        kv = proj(D, 3 * D, c0, c0 + PC)
        put_k(kv, c0)
        put_v(kv[D:, :], c0)

    def load_q(tq, gate=None):
        q = qT_s[tq, _h(0, DA), :]
        qc_s[...] = q
        qf = _up(q[QHI // 2:D // 2]).astype(F32)
        if gate is not None:
            qf = qf + (gate - gate)
        qf_s[pl.ds(QHI, D - QHI), :] = qf

    qrow = lax.broadcasted_iota(jnp.int32, (128, TQ), 0)

    def qweights(i):
        q = _up(qc_s[_h((i * HPI) // 4 * GW, 128), :]).astype(F32)
        js = [(i * HPI + k) % 4 for k in range(HPI)]
        return jnp.concatenate(
            [jnp.where((qrow >= DH * j) & (qrow < DH * (j + 1)), q, 0.0) for j in js], axis=1).astype(BF16)

    def prologue():
        pk = lambda r0, r1, c0, c1: proj(r0, r1, c0, c1).astype(BF16)
        pad = lambda n: jnp.zeros((DA - D, n), BF16)
        wait(grp_a)
        start(grp_c)
        start(grp_d)
        for c0 in range(W0, W1, 128):
            w_transpose(c0, 128)
        ln1(0, XA, True)
        proj_q(W0, D, 0, XA)
        k1 = pk(D, KA, 0, XA)
        wait(grp_b)
        for c0 in range(W1, 2 * D, 128):
            w_transpose(c0, 128)
        ln1(XA, XA + LW, True)
        k2 = pk(KA, W1, 0, XA)
        ln1(XA + LW, PC)
        put_k(jnp.concatenate([k1, k2, pk(W1, 2 * D, 0, XA), pad(XA)], axis=0), 0)
        k3 = pk(D, KS, XA, PC)
        wait(grp_c)
        start(grp_e)
        w_transpose(0, W0)
        k_table(0, TB1)
        put_k(jnp.concatenate([k3, pk(KS, 2 * D, XA, PC), pad(PC - XA)], axis=0), XA)
        proj_q(W0, D, XA, PC)
        proj_q(0, W0, 0, VS)
        wait(grp_d)
        start(grp_f)
        w_transpose(2 * D, D)
        proj_q(0, W0, VS, PC)
        k_table(TB1, TB2)
        ln1(PC, 2 * PC)
        put_v(proj(2 * D, 3 * D, 0, PC), 0)
        proj_kv(PC)
        wait(grp_e)
        ln1(2 * PC, 3 * PC)
        z = proj(0, D, PC, 2 * PC)
        k_table(TB2, D, z[0:1, 0:LW])
        put_q(z, 0, PC)
        ln1(3 * PC, 4 * PC)
        proj_kv(2 * PC)
        proj_q(0, D, 2 * PC, 3 * PC)
        proj_kv(3 * PC)
        proj_q(0, D, 3 * PC, 4 * PC)
        woT_s[...] = _pk(_pad_heads_rows(wo_s[...].astype(F32), jnp.zeros((HP - DH, D), F32)).astype(BF16).T)
        brow = lax.broadcasted_iota(jnp.int32, (DA - D, F), 0)
        w1_s[pl.ds(D, DA - D), :] = jnp.where(brow == 0, b1_s[...].astype(F32).reshape(1, F), 0.0).astype(BF16)
        w1T_s[...] = _pk(w1_s[...].T)
        b2c_s[...] = jnp.broadcast_to(b2_s[...].astype(F32).reshape(1, D), (LW, D)).T
        load_q(0)
        for i in range(PA):
            sv_s[i] = _dot(_up(k_s[(i * HPI) // 4, _h(0, NV), :]), qweights(i))
        wait(grp_f)

    bufs = (s0, s1, s2)
    h_s, hp_s = hbufs[:NG], hbufs[NG:]

    def out_copy(t, og):
        return pltpu.make_async_copy(out_s.at[t, pl.ds(og * OR, OR), :],
                                     out_hbm.at[0, pl.ds(og * OR, OR), pl.ds(pl.multiple_of(t * TQ, TQ), TQ)],
                                     sems.at[5])

    def tile(t):
        dz = [pl.multiple_of(dz_s[k], 16) for k in range(3)]
        st = {"m": {}, "pend": [], "ties": [], "fi": 0}

        nxt = jnp.minimum(t + 1, NT - 1)
        qn_s[pl.ds(zero, QLO), :] = _up(qT_s[nxt, _h(0, QLO), :]).astype(F32)
        units = [(i,) + _unit(u) + (i * NCH + u < NA,) for i in range(NI) for u in range(NCH)]
        units = units[NA:] + units[:NA]

        def vpu_unit(gate):
            i, lt, kg, ahead = units.pop(0)
            h = i * HPI + lt // NG
            if ("qv", i, lt, ahead) not in st:
                q_ref = qn_s if ahead else qf_s
                st["qv", i, lt, ahead] = jnp.concatenate(
                    [jnp.broadcast_to(q_ref[pl.ds(h * DH + d, 1), pl.ds(lt % NG * LW, LW)], (UK, LW))[None]
                     for d in range(DH)], axis=0)
            prod = kb_s[pl.ds(h * DH, DH), pl.ds(kg * UK, UK), :] * st["qv", i, lt, ahead]
            z0 = jnp.concatenate([gate - gate] * (UK // 8), axis=0)
            acc = jnp.sum(jnp.concatenate([z0[None], prod], axis=0), axis=0)
            sv_s[i, pl.ds(kg * UK, UK), pl.ds(lt * LW, LW)] = acc
            return jnp.minimum(jnp.min(acc.reshape(UK // 8, 8, LW), axis=0), LOWEST)

        def scores(a):
            i, c = a // NC, a % NC
            if c == 0:
                st["qm"] = qweights(i)
            k0, nk = MCH[c], MCH[c + 1] - MCH[c]
            s = _dot(_up(k_s[(i * HPI) // 4, _h(k0, nk), :]), st["qm"])
            bufs[i % 3][pl.ds(k0, nk), :] = s
            for lt in range(NLT):
                m = jnp.max(s[:, lt * LW:(lt + 1) * LW].reshape(nk // 8, 8, LW), axis=0)
                st["m8", lt] = m if c == 0 else jnp.maximum(m, st["m8", lt])
            pend = st["pend"]
            for r, lt in GATE.get(RATE[a], ()):
                pend.append((a + TD, (lt + 2) % NLT, vpu_unit(s[8 * r:8 * r + 8, lt * LW:(lt + 1) * LW])))
            while pend and pend[0][0] <= a:
                _, lt, v = pend.pop(0)
                st["m8", lt] = jnp.maximum(st["m8", lt], v)
            for u in range(c * NCH // NC, (c + 1) * NCH // NC):
                lt, kg = _unit(u)
                assert (i, lt, kg, False) not in units
                sv = sv_s[i, pl.ds(zero + kg * UK, UK), pl.ds(lt * LW, LW)]
                st["m8", lt] = jnp.maximum(st["m8", lt], jnp.max(sv.reshape(UK // 8, 8, LW), axis=0))
            if c == NC - 1:
                m8 = jnp.concatenate([st["m8", lt] for lt in range(NLT)], axis=1)
                st["m"][i] = jnp.max(m8, axis=0, keepdims=True)

        def probs_pv(i, k0, nk, q0, nq, first, last):
            for k in range(HPI):
                h = i * HPI + k
                lo = k * TQ + q0
                parts = []
                if k0 < NV:
                    parts.append(sv_s[i, pl.ds(zero + k0, min(NV - k0, nk)), pl.ds(lo, nq)])
                if k0 + nk > NV:
                    parts.append(bufs[i % 3][pl.ds(zero + max(k0, NV), k0 + nk - max(k0, NV)), pl.ds(lo, nq)])
                p = jnp.exp2(jnp.concatenate(parts, axis=0) - st["m"][i][:, lo:lo + nq])
                pv = _dot(_up(vT_s[_h(h * HP, HP), pl.ds(k0, nk)]), p.astype(BF16))
                acc = pv if first else st["acc", k] + pv
                st["acc", k] = acc
                if last:
                    l = acc[DH:DH + 1, :]
                    r = pl.reciprocal(l, approx=True)
                    r = r * (2.0 - l * r)
                    oT_s[_h(h * HP, HP), pl.ds(q0, nq)] = _pk((acc * r).astype(BF16))

        fcost = [T2, FCH[0][1] - T2, FCH[0][1]]
        for idx, (f0, fn) in enumerate(FCH):
            if idx < len(FCH) - 1:
                fcost += [2 * FCH[idx + 1][1], D * fn // 256]
            else:
                fcost += [OR * fn // 256] * (D // OR)
        fcost = [c * w for c, w in zip(fcost, FW)]
        fcum = [int(sum(fcost[:j]) * NA / sum(fcost) + 1e-6) for j in range(len(fcost) + 1)]

        def fdot(a, b):
            if b.shape[0] > 256 and b.shape[1] > LW:
                z = jnp.concatenate([_dot(a, b[:, l * LW:(l + 1) * LW]) for l in range(b.shape[1] // LW)], axis=1)
            else:
                z = _dot(a, b)
            n = fcum[st["fi"] + 1] - fcum[st["fi"]]
            st["fi"] += 1
            nr, nl = z.shape[0] // 8, z.shape[1] // LW
            ties = {}
            for pos, v in st["ties"]:
                ties.setdefault(min(pos, nr * nl - 1), []).append(v)
            st["ties"] = []
            blk = lambda pos: z[8 * (pos % nr):8 * (pos % nr) + 8, (pos // nr) * LW:(pos // nr + 1) * LW]
            for u in range(n):
                pos = u * nr * nl // n
                v = vpu_unit(blk(pos))
                if pos + FD < nr * nl:
                    ties.setdefault(pos + FD, []).append(v)
                else:
                    st["ties"].append((pos + FD - nr * nl, v))
            if not ties:
                return z
            cols = []
            for l in range(nl):
                parts, r0 = [], 0
                for pos in sorted(p for p in ties if p // nr == l):
                    r = pos % nr
                    if r > r0:
                        parts.append(z[8 * r0:8 * r, l * LW:(l + 1) * LW])
                    zb = blk(pos)
                    for v in ties[pos]:
                        zb = jnp.maximum(zb, v)
                    parts.append(zb)
                    r0 = r + 1
                if r0 < nr:
                    parts.append(z[8 * r0:, l * LW:(l + 1) * LW])
                cols.append(jnp.concatenate(parts, axis=0))
            return jnp.concatenate(cols, axis=1)

        def wo_part(cg, r):
            rows = pl.ds(r * UR, UR)
            hp = (xT_s[t, rows, pl.ds(cg * LW, LW)].astype(F32)
                  + _dot(_up(woT_s[_h(r * UR, UR), pl.ds(0, KP)]), _up(oT_s[_h(0, KP), pl.ds(cg * LW, LW)])))
            hp_s[cg][rows, :] = hp
            st["c", cg] = _fold(hp) if r == 0 else st["c", cg] + _fold(hp)

        def wo_last_ln2(cg):
            lc = pl.ds(cg * LW, LW)
            ol = _up(oT_s[_h(KP, H * HP - KP), lc])
            shift = jnp.sum(st["c", cg], axis=0, keepdims=True) * (1.0 / D)
            p1, p2 = [], []
            for r in range(4):
                hr = (hp_s[cg][pl.ds(dz[0] + r * GW, GW), :]
                      + _dot(_up(woT_s[_h(r * GW, GW), pl.ds(KP, H * HP - KP)]), ol))
                h_s[cg][pl.ds(r * GW, GW), :] = hr
                d = hr - shift
                p1.append(_fold(d))
                p2.append(_fold(d * d))
            dm = _colmean(p1)
            rs = lax.rsqrt(jnp.maximum(_colmean(p2) - dm * dm, 0.0) + EPS)
            mu = shift + dm
            for r in range(4):
                hn_s[_h(r * GW, GW), lc] = _pk(((h_s[cg][pl.ds(dz[2] + r * GW, GW), :] - mu) * rs).astype(BF16))

        def ffn1(f0, fn, cg=None):
            hn = hn_s[...] if cg is None else hn_s[:, pl.ds(cg * LW, LW)]
            a = jnp.maximum(fdot(_up(w1T_s[_h(f0, fn), :]), _up(hn)), 0.0)
            return a * a

        queue = [(cg, r) for cg in range(NG) for r in range(D // UR)]

        def fill(n):
            for _ in range(min(n, len(queue))):
                wo_part(*queue.pop(0))

        for a in range(NI * NC + LAG):
            b = a - NC - LAG
            if b >= 0:
                probs_pv(b // NC, (b + ROT) % NC * CK, CK, 0, TQ, b % NC == 0, b % NC == NC - 1)
            if a < NI * NC:
                scores(a)
            else:
                fill(1)
        nch = NC // NG
        for cg in range(NG):
            for c in range(nch):
                if cg > 0 and c == T1:
                    assert all(q[0] >= cg for q in queue)
                    wo_last_ln2(cg - 1)
                probs_pv(NI - 1, (c + ROT // NG) % nch * CK * NG, CK * NG, cg * LW, LW, c == 0, c == nch - 1)
                fill(FILL[cg * nch + c])
        fill(len(queue))
        f0, fn = FCH[0]
        a00 = ffn1(f0, T2, 0)
        wo_last_ln2(NG - 1)
        a01 = ffn1(f0 + T2, fn - T2, 0)
        a_next = jnp.concatenate([jnp.concatenate([a00, a01], axis=0), ffn1(f0, fn, 1)], axis=1)

        load_q(nxt, a_next[fn - 1:, :])
        b2c = b2c_s[...]
        acc = jnp.concatenate([h_s[cg][pl.ds(dz[0], D), :] + b2c for cg in range(NG)], axis=1)
        for i, (f0, fn) in enumerate(FCH):
            a = a_next.astype(BF16)
            if i < len(FCH) - 1:
                a_next = ffn1(*FCH[i + 1])
                acc = acc + fdot(w2T_s[:, pl.ds(f0, fn)], a)
            else:
                for og in range(D // OR):
                    res = acc[og * OR:(og + 1) * OR, :] + fdot(w2T_s[pl.ds(og * OR, OR), pl.ds(f0, fn)], a)
                    out_s[t, pl.ds(og * OR, OR), :] = res.astype(BF16)
                    out_copy(t, og).start()
        assert not units

    def step(i, carry):
        pl.when(i == 0)(prologue)
        pl.when(i > 0)(lambda: tile(i - 1))
        return carry

    lax.fori_loop(0, NT + 1, step, 0)
    for t in range(NT):
        for og in range(D // OR):
            out_copy(t, og).wait()


@jax.jit
def pallas_sequential_preLN__mha_block__dense_activation_squared_relu__prompt_kernel(
    A_x: jax.Array,
    A_wqkv: jax.Array,
    A_wo: jax.Array,
    B_x: jax.Array,
    B_w1: jax.Array,
    B_b1: jax.Array,
    B_w2: jax.Array,
    B_b2: jax.Array,
):
    del B_x
    hbm = pl.BlockSpec(memory_space=pltpu.HBM)
    outT = pl.pallas_call(
        _kernel,
        out_shape=jax.ShapeDtypeStruct((1, D, S), BF16),
        in_specs=[hbm] * 7,
        out_specs=hbm,
        scratch_shapes=[
            pltpu.VMEM((NT, D, TQ), BF16),
            pltpu.VMEM((D, 3 * D), BF16),
            pltpu.VMEM((D, D), BF16),
            pltpu.VMEM((DA, F), BF16),
            pltpu.VMEM((F,), BF16),
            pltpu.VMEM((D, F), BF16),
            pltpu.VMEM((D,), BF16),
            pltpu.VMEM((3 * D // 2, D), U32),
            pltpu.VMEM((D // 2, H * HP), U32),
            pltpu.VMEM((F // 2, DA), U32),
            pltpu.VMEM((D, LW), F32),
            pltpu.VMEM((D // 2, S), U32),
            pltpu.VMEM((4, S // 2, 128), U32),
            pltpu.VMEM((D, NV, 128), F32),
            pltpu.VMEM((NT, 256, TQ), U32),
            pltpu.VMEM((DA // 2, TQ), U32),
            pltpu.VMEM((D, TQ), F32),
            pltpu.VMEM((D, TQ), F32),
            pltpu.VMEM((H * HP // 2, S), U32),
            pltpu.VMEM((S, SW), F32),
            pltpu.VMEM((S, SW), F32),
            pltpu.VMEM((S, SW), F32),
            pltpu.VMEM((NI, NV, SW), F32),
            pltpu.VMEM((H * HP // 2, TQ), U32),
            pltpu.VMEM((DA // 2, TQ), U32),
            pltpu.VMEM((NT, D, TQ), BF16),
            pltpu.SMEM((3,), jnp.int32),
            pltpu.SMEM((3,), jnp.int32),
            pltpu.SemaphoreType.DMA((6,)),
        ] + [pltpu.VMEM((D, LW), F32)] * (2 * NG),
        compiler_params=pltpu.CompilerParams(vmem_limit_bytes=100 * 1024 * 1024,
                                             disable_bounds_checks=True,
                                             disable_semaphore_checks=True),
        name="fused_block",
    )(jnp.transpose(A_x, (0, 2, 1)), A_wqkv, A_wo, B_w1, B_b1, B_w2.T, B_b2)
    return jnp.transpose(outT, (0, 2, 1))
```

```python
import jax
import jax.numpy as jnp
from jax import lax
import jax.experimental.pallas as pl
import jax.experimental.pallas.tpu as pltpu

S, D, H, DH, F = 2048, 448, 16, 28, 1792
HP = 32
GW = 4 * DH
DA = 464
PC = 512
TQ = 256
NT = S // TQ
HPI = 2
NI = H // HPI
IR = HPI * DH
SW = HPI * TQ
CK = 128
NC = S // CK
LAG = 3
LW = 128
NG = TQ // LW
NLT = SW // LW
KP = 3 * 128
UR = 64
FCH = ((0, 512), (512, 512), (1024, 512), (1536, 256))
OR = 224
FILL = (0, 1, 0, 1, 1, 1, 0, 0, 1, 1, 1, 0, 0, 1, 0, 1)
T1, T2, ROT = 5, 160, 4
W0, W1, XA = 384, 640, 256
KA, KS, VS = 576, 720, 384
TB1, TB2 = 23, 160
NV, UK = 192, 16
NKG = NV // UK
NCH = NLT * NKG
RA = (2, 2, 2, 2, 2, 3, 3) + (2,) * 12
RP = (2, 1, 2, 2, 3, 1, 2, 2, 3, 1, 2, 2, 2, 2, 2, 2)
RATE = [RA[a] if a < NC + LAG else (RP[a % NC] if a < NI * NC - 4 else 0) for a in range(NI * NC)]
GATE = {1: ((8, 0),), 2: ((1, 0), (7, 2)), 3: ((1, 0), (5, 2), (10, 2))}
NA = NI * NCH - sum(RATE)
PA, PL = -(-NA // NCH), NA // NCH
QLO, QHI = -(-PA * HPI * DH // 16) * 16, PL * HPI * DH // 16 * 16
FW = (0, 0.7, 1, 1, 1.15, 1, 1, 1, 1, 0.5, 0.15)
TD, FD = 2, 32
MCH = [NV + 16 * (c * ((S - NV) // 16) // NC) for c in range(NC + 1)]
EPS = 1e-5
QSCALE = (DH ** -0.5) * 1.4426950408889634
LOWEST = -3.0e38
F32 = jnp.float32
BF16 = jnp.bfloat16
U32 = jnp.uint32


def _pad_heads_rows(m, filler):
    parts = []
    for h in range(H):
        parts.append(m[DH * h:DH * (h + 1), :])
        parts.append(filler)
    return jnp.concatenate(parts, axis=0)


def _fold(v):
    v = jnp.sum(v.reshape(v.shape[0] // 16, 16, v.shape[1]), axis=0)
    return v[:8] + v[8:]


def _colmean(parts):
    return jnp.sum((parts[0] + parts[1]) + (parts[2] + parts[3]), axis=0, keepdims=True) * (1.0 / D)


def _pk(x):
    return pltpu.bitcast(x, U32)


def _up(x):
    return pltpu.bitcast(x, BF16)


def _h(start, size):
    return pl.ds(start // 2, size // 2)


def _dot(a, b):
    return jnp.dot(a, b, preferred_element_type=F32)


def _unit(u):
    return u % NLT, (u // NLT + 5 * (u % NLT)) % NKG


def _kernel(xT_hbm, wqkv_hbm, wo_hbm, w1_hbm, b1_hbm, w2T_hbm, b2_hbm, out_hbm,
            xT_s, wqkv_s, wo_s, w1_s, b1_s, w2T_s, b2_s,
            wT_s, woT_s, w1T_s, b2c_s, xn_s,
            k_s, qT_s, qc_s, vT_s, s0, s1, s2, oT_s, hn_s, out_s,
            zero_s, sems, h_s, hp_s, kb_s, qf_s, qn_s, sv_s):
    def w_copy(c0, n, sem):
        return pltpu.make_async_copy(wqkv_hbm.at[:, pl.ds(c0, n)], wqkv_s.at[:, pl.ds(c0, n)], sems.at[sem])

    def x_copy(c0, n, sem):
        return [pltpu.make_async_copy(xT_hbm.at[0, :, pl.ds(c, TQ)], xT_s.at[c // TQ], sems.at[sem])
                for c in range(c0, c0 + n, TQ)]

    grp_a = [w_copy(W0, W1 - W0, 0)] + x_copy(0, XA, 0)
    grp_b = x_copy(XA, PC - XA, 1) + [w_copy(W1, 2 * D - W1, 1)]
    grp_c = [w_copy(0, W0, 3)]
    grp_d = [w_copy(2 * D, D, 2)] + x_copy(PC, PC, 2)
    grp_e = x_copy(2 * PC, 2 * PC, 4) + [
             pltpu.make_async_copy(wo_hbm, wo_s, sems.at[4]),
             pltpu.make_async_copy(w1_hbm, w1_s.at[pl.ds(0, D), :], sems.at[4]),
             pltpu.make_async_copy(b1_hbm, b1_s, sems.at[4]),
             pltpu.make_async_copy(b2_hbm, b2_s, sems.at[4])]
    grp_f = [pltpu.make_async_copy(w2T_hbm, w2T_s, sems.at[0])]

    def start(grp):
        for cp in grp:
            cp.start()

    def wait(grp):
        for cp in grp:
            cp.wait()

    start(grp_a)
    start(grp_b)
    for k in range(3):
        zero_s[k] = 0
    zeros0 = [pl.multiple_of(lax.shift_right_logical(jnp.clip(zero_s[k], 0, 7), 3), 16) for k in range(3)]
    zero = zeros0[0]
    qT_s[:, _h(D, DA - D), :] = jnp.zeros((NT, (DA - D) // 2, TQ), U32)
    arow = lax.broadcasted_iota(jnp.int32, (DA - D, TQ), 0)
    hn_s[_h(D, DA - D), :] = _pk(jnp.where(arow == 0, 1.0, 0.0).astype(BF16))

    def ln1(c0, c1, zeros, split=False):
        for cg in range(c0 // LW, c1 // LW):
            cols = pl.ds(cg * LW, LW)
            xt, xc = cg // NG, pl.ds(cg % NG * LW, LW)
            if split:
                ld = lambda k, r: xT_s[xt, pl.ds(zeros[k] + r * GW, GW), xc].astype(F32)
                mu = _colmean([_fold(ld(0, r)) for r in range(4)])
                var = _colmean([_fold(jnp.square(ld(1, r) - mu)) for r in range(4)])
                rs = lax.rsqrt(var + EPS)
                for r in range(4):
                    xn_s[_h(r * GW, GW), cols] = _pk(((ld(2, r) - mu) * rs).astype(BF16))
            else:
                ld = lambda k: xT_s[xt, pl.ds(zeros[k], D), xc].astype(F32)
                mu = jnp.sum(ld(0), axis=0, keepdims=True) * (1.0 / D)
                var = jnp.sum(jnp.square(ld(1) - mu), axis=0, keepdims=True) * (1.0 / D)
                xn_s[:, cols] = _pk(((ld(2) - mu) * lax.rsqrt(var + EPS)).astype(BF16))

    def w_transpose(c0, n):
        wT_s[_h(c0, n), :] = _pk(wqkv_s[:, pl.ds(c0, n)].T)

    def k_table(d0, d1, gate=None):
        for g in range(4):
            if max(d0, g * GW) >= min(d1, (g + 1) * GW):
                continue
            kp = k_s[g, pl.ds(zero, NV // 2), :]
            if gate is not None:
                kp = kp | pltpu.bitcast(gate - gate, U32)
            for i in range(g * 4 // HPI, (g + 1) * 4 // HPI):
                lo, hi = max(d0, i * IR), min(d1, (i + 1) * IR)
                if lo < hi:
                    kb_s[i][pl.ds(lo - i * IR, hi - lo)] = jnp.concatenate(
                        [_up(jnp.broadcast_to(kp[:, d - g * GW:d - g * GW + 1], (NV // 2, 128))).astype(F32)[None]
                         for d in range(lo, hi)], axis=0)

    def proj(r0, r1, c0, c1):
        xr = pl.ds(zero if c0 >= PC else 0, D // 2)
        return _dot(_up(wT_s[_h(r0, r1 - r0), :]), _up(xn_s[xr, pl.ds(c0, c1 - c0)]))

    def put_q(z, r0, c0):
        c = c0
        while c < c0 + z.shape[1]:
            n = min(TQ - c % TQ, c0 + z.shape[1] - c)
            qT_s[c // TQ, _h(r0, z.shape[0]), pl.ds(c % TQ, n)] = _pk((z[:, c - c0:c - c0 + n] * QSCALE).astype(BF16))
            c += n

    def put_k(kT, c0):
        for g in range(4):
            k_s[g, _h(c0, kT.shape[1]), :] = _pk(kT[GW * g:GW * g + 128, :].astype(BF16).T)

    def put_v(vT, c0):
        ones_row = jnp.where(lax.broadcasted_iota(jnp.int32, (HP - DH, PC), 0) == 0, 1.0, 0.0)
        vT_s[:, pl.ds(c0, PC)] = _pk(_pad_heads_rows(vT, ones_row).astype(BF16))

    def proj_q(r0, r1, c0, c1):
        put_q(proj(r0, r1, c0, c1), r0, c0)

    def proj_kv(c0):
        kv = proj(D, 3 * D, c0, c0 + PC)
        put_k(kv, c0)
        put_v(kv[D:, :], c0)

    def load_q(tq, gate=None):
        q = qT_s[tq, _h(0, DA), :]
        qc_s[...] = q
        qf = _up(q[QHI // 2:D // 2]).astype(F32)
        if gate is not None:
            qf = qf + (gate - gate)
        for i in range(PL, NI):
            qf_s[i - PL][...] = qf[i * IR - QHI:(i + 1) * IR - QHI]

    qrow = lax.broadcasted_iota(jnp.int32, (128, TQ), 0)

    def qweights(i):
        q = _up(qc_s[_h((i * HPI) // 4 * GW, 128), :]).astype(F32)
        js = [(i * HPI + k) % 4 for k in range(HPI)]
        return jnp.concatenate(
            [jnp.where((qrow >= DH * j) & (qrow < DH * (j + 1)), q, 0.0) for j in js], axis=1).astype(BF16)

    def prologue(dz):
        pk = lambda r0, r1, c0, c1: proj(r0, r1, c0, c1).astype(BF16)
        pad = lambda n: jnp.zeros((DA - D, n), BF16)
        wait(grp_a)
        start(grp_c)
        start(grp_d)
        for c0 in range(W0, W1, 128):
            w_transpose(c0, 128)
        ln1(0, XA, zeros0, True)
        proj_q(W0, D, 0, XA)
        k1 = pk(D, KA, 0, XA)
        wait(grp_b)
        for c0 in range(W1, 2 * D, 128):
            w_transpose(c0, 128)
        ln1(XA, XA + LW, zeros0, True)
        k2 = pk(KA, W1, 0, XA)
        ln1(XA + LW, PC, dz)
        put_k(jnp.concatenate([k1, k2, pk(W1, 2 * D, 0, XA), pad(XA)], axis=0), 0)
        k3 = pk(D, KS, XA, PC)
        wait(grp_c)
        start(grp_e)
        w_transpose(0, W0)
        k_table(0, TB1)
        put_k(jnp.concatenate([k3, pk(KS, 2 * D, XA, PC), pad(PC - XA)], axis=0), XA)
        proj_q(W0, D, XA, PC)
        proj_q(0, W0, 0, VS)
        wait(grp_d)
        start(grp_f)
        w_transpose(2 * D, D)
        proj_q(0, W0, VS, PC)
        k_table(TB1, TB2)
        ln1(PC, 2 * PC, dz)
        put_v(proj(2 * D, 3 * D, 0, PC), 0)
        proj_kv(PC)
        wait(grp_e)
        ln1(2 * PC, 3 * PC, dz)
        z = proj(0, D, PC, 2 * PC)
        k_table(TB2, D, z[0:1, 0:LW])
        put_q(z, 0, PC)
        ln1(3 * PC, 4 * PC, dz)
        proj_kv(2 * PC)
        proj_q(0, D, 2 * PC, 3 * PC)
        proj_kv(3 * PC)
        proj_q(0, D, 3 * PC, 4 * PC)
        woT_s[...] = _pk(_pad_heads_rows(wo_s[...].astype(F32), jnp.zeros((HP - DH, D), F32)).astype(BF16).T)
        brow = lax.broadcasted_iota(jnp.int32, (DA - D, F), 0)
        w1_s[pl.ds(D, DA - D), :] = jnp.where(brow == 0, b1_s[...].astype(F32).reshape(1, F), 0.0).astype(BF16)
        w1T_s[...] = _pk(w1_s[...].T)
        b2c_s[...] = jnp.broadcast_to(b2_s[...].astype(F32).reshape(1, D), (LW, D)).T
        load_q(0)
        for i in range(PA):
            sv_s[i][...] = _dot(_up(k_s[(i * HPI) // 4, _h(0, NV), :]), qweights(i))
        wait(grp_f)

    bufs = (s0, s1, s2)

    def out_copy(t, og):
        return pltpu.make_async_copy(out_s.at[t, pl.ds(og * OR, OR), :],
                                     out_hbm.at[0, pl.ds(og * OR, OR), pl.ds(pl.multiple_of(t * TQ, TQ), TQ)],
                                     sems.at[5])

    def tile(t, dz):
        st = {"m": {}, "pend": [], "ties": [], "fi": 0}

        nxt = jnp.minimum(t + 1, NT - 1)
        qn = _up(qT_s[nxt, _h(0, QLO), :]).astype(F32)
        for i in range(PA):
            qn_s[i][pl.ds(zero, IR), :] = qn[i * IR:(i + 1) * IR]
        units = [(i,) + _unit(u) + (i * NCH + u < NA,) for i in range(NI) for u in range(NCH)]
        units = units[NA:] + units[:NA]

        def vpu_unit(gate):
            i, lt, kg, ahead = units.pop(0)
            r0 = lt // NG * DH
            if ("qv", i, lt, ahead) not in st:
                q_ref = qn_s[i] if ahead else qf_s[i - PL]
                st["qv", i, lt, ahead] = jnp.concatenate(
                    [jnp.broadcast_to(q_ref[pl.ds(r0 + d, 1), pl.ds(lt % NG * LW, LW)], (UK, LW))[None]
                     for d in range(DH)], axis=0)
            prod = kb_s[i][pl.ds(r0, DH), pl.ds(kg * UK, UK), :] * st["qv", i, lt, ahead]
            z0 = jnp.concatenate([gate - gate] * (UK // 8), axis=0)
            acc = jnp.sum(jnp.concatenate([z0[None], prod], axis=0), axis=0)
            sv_s[i][pl.ds(kg * UK, UK), pl.ds(lt * LW, LW)] = acc
            return jnp.minimum(jnp.min(acc.reshape(UK // 8, 8, LW), axis=0), LOWEST)

        def scores(a):
            i, c = a // NC, a % NC
            if c == 0:
                st["qm"] = qweights(i)
            k0, nk = MCH[c], MCH[c + 1] - MCH[c]
            s = _dot(_up(k_s[(i * HPI) // 4, _h(k0, nk), :]), st["qm"])
            bufs[i % 3][pl.ds(k0, nk), :] = s
            for lt in range(NLT):
                m = jnp.max(s[:, lt * LW:(lt + 1) * LW].reshape(nk // 8, 8, LW), axis=0)
                st["m8", lt] = m if c == 0 else jnp.maximum(m, st["m8", lt])
            pend = st["pend"]
            for r, lt in GATE.get(RATE[a], ()):
                pend.append((a + TD, (lt + 2) % NLT, vpu_unit(s[8 * r:8 * r + 8, lt * LW:(lt + 1) * LW])))
            while pend and pend[0][0] <= a:
                _, lt, v = pend.pop(0)
                st["m8", lt] = jnp.maximum(st["m8", lt], v)
            for u in range(c * NCH // NC, (c + 1) * NCH // NC):
                lt, kg = _unit(u)
                assert (i, lt, kg, False) not in units
                sv = sv_s[i][pl.ds(zero + kg * UK, UK), pl.ds(lt * LW, LW)]
                st["m8", lt] = jnp.maximum(st["m8", lt], jnp.max(sv.reshape(UK // 8, 8, LW), axis=0))
            if c == NC - 1:
                m8 = jnp.concatenate([st["m8", lt] for lt in range(NLT)], axis=1)
                st["m"][i] = jnp.max(m8, axis=0, keepdims=True)

        def probs_pv(i, k0, nk, q0, nq, first, last):
            for k in range(HPI):
                h = i * HPI + k
                lo = k * TQ + q0
                parts = []
                if k0 < NV:
                    parts.append(sv_s[i][pl.ds(zero + k0, min(NV - k0, nk)), pl.ds(lo, nq)])
                if k0 + nk > NV:
                    parts.append(bufs[i % 3][pl.ds(zero + max(k0, NV), k0 + nk - max(k0, NV)), pl.ds(lo, nq)])
                p = jnp.exp2(jnp.concatenate(parts, axis=0) - st["m"][i][:, lo:lo + nq])
                pv = _dot(_up(vT_s[_h(h * HP, HP), pl.ds(k0, nk)]), p.astype(BF16))
                acc = pv if first else st["acc", k] + pv
                st["acc", k] = acc
                if last:
                    l = acc[DH:DH + 1, :]
                    r = pl.reciprocal(l, approx=True)
                    r = r * (2.0 - l * r)
                    oT_s[_h(h * HP, HP), pl.ds(q0, nq)] = _pk((acc * r).astype(BF16))

        fcost = [T2, FCH[0][1] - T2, FCH[0][1]]
        for idx, (f0, fn) in enumerate(FCH):
            if idx < len(FCH) - 1:
                fcost += [2 * FCH[idx + 1][1], D * fn // 256]
            else:
                fcost += [OR * fn // 256] * (D // OR)
        fcost = [c * w for c, w in zip(fcost, FW)]
        fcum = [int(sum(fcost[:j]) * NA / sum(fcost) + 1e-6) for j in range(len(fcost) + 1)]

        def fdot(a, b):
            if b.shape[0] > 256 and b.shape[1] > LW:
                z = jnp.concatenate([_dot(a, b[:, l * LW:(l + 1) * LW]) for l in range(b.shape[1] // LW)], axis=1)
            else:
                z = _dot(a, b)
            n = fcum[st["fi"] + 1] - fcum[st["fi"]]
            st["fi"] += 1
            nr, nl = z.shape[0] // 8, z.shape[1] // LW
            ties = {}
            for pos, v in st["ties"]:
                ties.setdefault(min(pos, nr * nl - 1), []).append(v)
            st["ties"] = []
            blk = lambda pos: z[8 * (pos % nr):8 * (pos % nr) + 8, (pos // nr) * LW:(pos // nr + 1) * LW]
            for u in range(n):
                pos = u * nr * nl // n
                v = vpu_unit(blk(pos))
                if pos + FD < nr * nl:
                    ties.setdefault(pos + FD, []).append(v)
                else:
                    st["ties"].append((pos + FD - nr * nl, v))
            if not ties:
                return z
            cols = []
            for l in range(nl):
                parts, r0 = [], 0
                for pos in sorted(p for p in ties if p // nr == l):
                    r = pos % nr
                    if r > r0:
                        parts.append(z[8 * r0:8 * r, l * LW:(l + 1) * LW])
                    zb = blk(pos)
                    for v in ties[pos]:
                        zb = jnp.maximum(zb, v)
                    parts.append(zb)
                    r0 = r + 1
                if r0 < nr:
                    parts.append(z[8 * r0:, l * LW:(l + 1) * LW])
                cols.append(jnp.concatenate(parts, axis=0))
            return jnp.concatenate(cols, axis=1)

        def wo_part(cg, r):
            rows = pl.ds(r * UR, UR)
            hp = (xT_s[t, rows, pl.ds(cg * LW, LW)].astype(F32)
                  + _dot(_up(woT_s[_h(r * UR, UR), pl.ds(0, KP)]), _up(oT_s[_h(0, KP), pl.ds(cg * LW, LW)])))
            hp_s[cg][rows, :] = hp
            st["c", cg] = _fold(hp) if r == 0 else st["c", cg] + _fold(hp)

        def wo_last_ln2(cg):
            lc = pl.ds(cg * LW, LW)
            ol = _up(oT_s[_h(KP, H * HP - KP), lc])
            shift = jnp.sum(st["c", cg], axis=0, keepdims=True) * (1.0 / D)
            p1, p2 = [], []
            for r in range(4):
                hr = (hp_s[cg][pl.ds(dz[0] + r * GW, GW), :]
                      + _dot(_up(woT_s[_h(r * GW, GW), pl.ds(KP, H * HP - KP)]), ol))
                h_s[cg][pl.ds(r * GW, GW), :] = hr
                d = hr - shift
                p1.append(_fold(d))
                p2.append(_fold(d * d))
            dm = _colmean(p1)
            rs = lax.rsqrt(jnp.maximum(_colmean(p2) - dm * dm, 0.0) + EPS)
            mu = shift + dm
            for r in range(4):
                hn_s[_h(r * GW, GW), lc] = _pk(((h_s[cg][pl.ds(dz[2] + r * GW, GW), :] - mu) * rs).astype(BF16))

        def ffn1(f0, fn, cg=None):
            hn = hn_s[...] if cg is None else hn_s[:, pl.ds(cg * LW, LW)]
            a = jnp.maximum(fdot(_up(w1T_s[_h(f0, fn), :]), _up(hn)), 0.0)
            return a * a

        queue = [(cg, r) for cg in range(NG) for r in range(D // UR)]

        def fill(n):
            for _ in range(min(n, len(queue))):
                wo_part(*queue.pop(0))

        for a in range(NI * NC + LAG):
            b = a - NC - LAG
            if b >= 0:
                probs_pv(b // NC, (b + ROT) % NC * CK, CK, 0, TQ, b % NC == 0, b % NC == NC - 1)
            if a < NI * NC:
                scores(a)
            else:
                fill(1)
        nch = NC // NG
        for cg in range(NG):
            for c in range(nch):
                if cg > 0 and c == T1:
                    assert all(q[0] >= cg for q in queue)
                    wo_last_ln2(cg - 1)
                probs_pv(NI - 1, (c + ROT // NG) % nch * CK * NG, CK * NG, cg * LW, LW, c == 0, c == nch - 1)
                fill(FILL[cg * nch + c])
        fill(len(queue))
        f0, fn = FCH[0]
        a00 = ffn1(f0, T2, 0)
        wo_last_ln2(NG - 1)
        a01 = ffn1(f0 + T2, fn - T2, 0)
        a_next = jnp.concatenate([jnp.concatenate([a00, a01], axis=0), ffn1(f0, fn, 1)], axis=1)

        load_q(nxt, a_next[fn - 1:, :])
        b2c = b2c_s[...]
        acc = jnp.concatenate([h_s[cg][pl.ds(dz[0], D), :] + b2c for cg in range(NG)], axis=1)
        for i, (f0, fn) in enumerate(FCH):
            a = a_next.astype(BF16)
            if i < len(FCH) - 1:
                a_next = ffn1(*FCH[i + 1])
                acc = acc + fdot(w2T_s[:, pl.ds(f0, fn)], a)
            else:
                for og in range(D // OR):
                    res = acc[og * OR:(og + 1) * OR, :] + fdot(w2T_s[pl.ds(og * OR, OR), pl.ds(f0, fn)], a)
                    out_s[t, pl.ds(og * OR, OR), :] = res.astype(BF16)
                    out_copy(t, og).start()
        assert not units

    def step(i, carry):
        dz = [pl.multiple_of(lax.shift_right_logical(i, 4 + k), 16) for k in range(3)]
        pl.when(i == 0)(lambda: prologue(dz))
        pl.when(i > 0)(lambda: tile(i - 1, dz))
        return carry

    lax.fori_loop(0, NT + 1, step, 0)
    for t in range(NT):
        for og in range(D // OR):
            out_copy(t, og).wait()


@jax.jit
def pallas_sequential_preLN__mha_block__dense_activation_squared_relu__prompt_kernel(
    A_x: jax.Array,
    A_wqkv: jax.Array,
    A_wo: jax.Array,
    B_x: jax.Array,
    B_w1: jax.Array,
    B_b1: jax.Array,
    B_w2: jax.Array,
    B_b2: jax.Array,
):
    del B_x
    hbm = pl.BlockSpec(memory_space=pltpu.HBM)
    outT = pl.pallas_call(
        _kernel,
        out_shape=jax.ShapeDtypeStruct((1, D, S), BF16),
        in_specs=[hbm] * 7,
        out_specs=hbm,
        scratch_shapes=[
            pltpu.VMEM((NT, D, TQ), BF16),
            pltpu.VMEM((D, 3 * D), BF16),
            pltpu.VMEM((D, D), BF16),
            pltpu.VMEM((DA, F), BF16),
            pltpu.VMEM((F,), BF16),
            pltpu.VMEM((D, F), BF16),
            pltpu.VMEM((D,), BF16),
            pltpu.VMEM((3 * D // 2, D), U32),
            pltpu.VMEM((D // 2, H * HP), U32),
            pltpu.VMEM((F // 2, DA), U32),
            pltpu.VMEM((D, LW), F32),
            pltpu.VMEM((D // 2, S), U32),
            pltpu.VMEM((4, S // 2, 128), U32),
            pltpu.VMEM((NT, 256, TQ), U32),
            pltpu.VMEM((DA // 2, TQ), U32),
            pltpu.VMEM((H * HP // 2, S), U32),
            pltpu.VMEM((S, SW), F32),
            pltpu.VMEM((S, SW), F32),
            pltpu.VMEM((S, SW), F32),
            pltpu.VMEM((H * HP // 2, TQ), U32),
            pltpu.VMEM((DA // 2, TQ), U32),
            pltpu.VMEM((NT, D, TQ), BF16),
            pltpu.SMEM((3,), jnp.int32),
            pltpu.SemaphoreType.DMA((6,)),
            [pltpu.VMEM((D, LW), F32)] * NG,
            [pltpu.VMEM((D, LW), F32)] * NG,
            [pltpu.VMEM((IR, NV, 128), F32)] * NI,
            [pltpu.VMEM((IR, TQ), F32)] * (NI - PL),
            [pltpu.VMEM((IR, TQ), F32)] * PA,
            [pltpu.VMEM((NV, SW), F32)] * NI,
        ],
        compiler_params=pltpu.CompilerParams(vmem_limit_bytes=100 * 1024 * 1024,
                                             disable_bounds_checks=True,
                                             disable_semaphore_checks=True),
        name="fused_block",
    )(jnp.transpose(A_x, (0, 2, 1)), A_wqkv, A_wo, B_w1, B_b1, B_w2.T, B_b2)
    return jnp.transpose(outT, (0, 2, 1))
```
